```python
import os as _os
_os.environ.setdefault("JAX_PLATFORMS", "cpu")
import jax
import jax.numpy as jnp

def _softmax(x, axis=-1):
    return jax.nn.softmax(x, axis=axis)
def _gelu(x):
    return jax.nn.gelu(x, approximate=True)
def _silu(x):
    return jax.nn.silu(x)
def _sigmoid(x):
    return jax.nn.sigmoid(x)
def _layernorm(x, axis=-1, eps=1e-5):
    m = jnp.mean(x, axis=axis, keepdims=True)
    v = jnp.var(x, axis=axis, keepdims=True)
    return (x - m) / jnp.sqrt(v + eps)
def _scatter_add(tgt, idx, src, axis=0):
    return tgt.at[idx].add(src)
def _segment_sum(src, seg, n):
    return jax.ops.segment_sum(src, seg, n)
class _Rng:
    def __init__(self, key):
        self._k = key
    def _next(self):
        self._k, sub = jax.random.split(self._k)
        return sub
    def normal(self, shape):
        return jax.random.normal(self._next(), shape, dtype=jnp.bfloat16)
    def randint(self, lo, hi, shape):
        return jax.random.randint(self._next(), shape, lo, hi, dtype=jnp.int32)
    def uniform(self, shape, lo=0.0, hi=1.0):
        return jax.random.uniform(self._next(), shape, jnp.bfloat16, lo, hi)
    def permutation(self, n):
        return jax.random.permutation(self._next(), n)


kernel_name = 'sequential_preLN__softmax_full_mha__mixer_channel_mlp__prompt'

def setup_inputs():
    _rng = _Rng(jax.random.key(int.from_bytes(__import__("os").urandom(4), "little")))
    _w = (lambda a: (lambda t: t.astype(jnp.bfloat16) if jnp.issubdtype(t.dtype, jnp.floating) else t)(jnp.asarray(a)))
    def _A_setup():
        B, S, D = 1, 2048, 1024
        return {
            "x": _w((lambda *s: _rng.normal(s) * 0.05)(B, S, D)),
            "wqkv": _w((lambda *s: _rng.normal(s) * 0.05)(D, 3 * D)),
            "wo": _w((lambda *s: _rng.normal(s) * 0.05)(D, D)),
        }
    _A_in = _A_setup()

    def _B_setup():
        B, S, D, F = 1, 2048, 1024, 3584
        return {
            "x": _w((lambda *s: _rng.normal(s) * 0.05)(B, S, D)),
            "w1": _w((lambda *s: _rng.normal(s) * 0.8)(D, F) * (D ** -0.5)),
            "b1": _w((lambda *s: _rng.normal(s) * 0.8)(F)),
            "w2": _w((lambda *s: _rng.normal(s) * 0.8)(F, D) * (F ** -0.5)),
            "b2": _w((lambda *s: _rng.normal(s) * 0.05)(D)),
        }
    _B_in = _B_setup()

    return {
        "A_x": _A_in["x"],
        "A_wqkv": _A_in["wqkv"],
        "A_wo": _A_in["wo"],
        "B_x": _B_in["x"],
        "B_w1": _B_in["w1"],
        "B_b1": _B_in["b1"],
        "B_w2": _B_in["w2"],
        "B_b2": _B_in["b2"],
    }

def reference(A_x, A_wqkv, A_wo, B_x, B_w1, B_b1, B_w2, B_b2):
    def _A_ref(x, wqkv, wo):
        B, S, D = x.shape
        H = 32; Dh = D // H
        qkv = (lambda x, *d: x.transpose(*d))((x @ wqkv).reshape(B, S, 3, H, Dh), 2, 0, 3, 1, 4)
        q, k, v = qkv[0], qkv[1], qkv[2]
        scale = Dh ** -0.5
        scores = jnp.einsum("bhqd,bhkd->bhqk", q, k) * scale
        p = _softmax(scores, axis=-1)
        o = jnp.einsum("bhqk,bhkd->bhqd", p, v)
        return (lambda x, *d: x.transpose(*d))(o, 0, 2, 1, 3).reshape(B, S, D) @ wo

    def _B_ref(x, w1, b1, w2, b2):
        y = _layernorm(x, axis=-1)
        h = _gelu(jnp.einsum("bsd,df->bsf", y, w1) + b1)
        return jnp.einsum("bsf,fd->bsd", h, w2) + b2

    x = A_x
    h = x + _A_ref(_layernorm(x, axis=-1), A_wqkv, A_wo)
    h2 = h + _B_ref(_layernorm(h, axis=-1), B_w1, B_b1, B_w2, B_b2)
    return h2
```

```python
import functools
import math

import jax
import jax.numpy as jnp
from jax import lax
import jax.experimental.pallas as pl
import jax.experimental.pallas.tpu as pltpu

_EPS = 1e-5
_H = 32
_TM1 = 512
_TQ = 1024
_NSUB = 8
_TM3 = 512
_FC = 512


def _layernorm(x):
    m = jnp.mean(x, axis=-1, keepdims=True)
    xc = x - m
    v = jnp.mean(xc * xc, axis=-1, keepdims=True)
    return xc * lax.rsqrt(v + _EPS)


def _kernel(x_hbm, wqkv_hbm, wo_hbm, w1_hbm, b1_hbm, w2_hbm, b2_hbm, out_hbm,
            x_v, wqkv_v, wo_v, w1_v, b1_v, w2_v, b2_v,
            qt_s, k_s, vt_s, ot_s, s_a, s_b, m_a, m_b, g_s, out_v,
            sem_x, sem_w, sem_o, *, S, D, F):
    f32, bf16 = jnp.float32, jnp.bfloat16
    Dh = D // _H
    n1 = S // _TM1
    n3 = S // _TM3

    def x_copy(i):
        return pltpu.make_async_copy(
            x_hbm.at[0, pl.ds(i * _TM1, _TM1), :],
            x_v.at[pl.ds(i * _TM1, _TM1), :], sem_x.at[i])

    def wqkv_copy(i):
        return pltpu.make_async_copy(
            wqkv_hbm.at[:, pl.ds(i * D, D)], wqkv_v.at[:, pl.ds(i * D, D)],
            sem_w.at[i])

    wo_copy = pltpu.make_async_copy(wo_hbm, wo_v, sem_w.at[3])
    w1_copy = pltpu.make_async_copy(w1_hbm, w1_v, sem_w.at[4])
    w2_copy = pltpu.make_async_copy(w2_hbm, w2_v, sem_w.at[5])
    b1_copy = pltpu.make_async_copy(b1_hbm, b1_v, sem_w.at[6])
    b2_copy = pltpu.make_async_copy(b2_hbm, b2_v, sem_w.at[7])

    x_copy(0).start()
    for i in range(3):
        wqkv_copy(i).start()
    for i in range(1, n1):
        x_copy(i).start()
    wo_copy.start()
    w1_copy.start()
    w2_copy.start()
    b1_copy.start()
    b2_copy.start()

    qscale = (Dh ** -0.5) * math.log2(math.e)

    for i in range(3):
        wqkv_copy(i).wait()

    def phase1(i, carry):
        x_copy(i).wait()
        r0 = pl.multiple_of(i * _TM1, _TM1)
        rows = pl.ds(r0, _TM1)
        y = _layernorm(x_v[rows, :].astype(f32)).astype(bf16)
        q = jnp.dot(y, wqkv_v[:, 0:D], preferred_element_type=f32) * qscale
        qt_s[:, rows] = q.T.astype(bf16)
        k = jnp.dot(y, wqkv_v[:, D:2 * D], preferred_element_type=f32)
        k_s[rows, :] = k.astype(bf16)
        v = jnp.dot(y, wqkv_v[:, 2 * D:3 * D], preferred_element_type=f32)
        vt_s[:, rows] = v.T.astype(bf16)
        return carry

    lax.fori_loop(0, n1, phase1, 0)

    NC = _TQ // 128
    KC = S // _NSUB
    kp = _NSUB // NC
    KP = S // kp
    NU = (S // _TQ) * _H

    def qk_weights(qb, g, j):
        qh = qt_s[pl.ds(pl.multiple_of(g * 128 + j * Dh, Dh), Dh),
                  pl.ds(pl.multiple_of(qb * _TQ, _TQ), _TQ)]
        parts = []
        if j > 0:
            parts.append(jnp.zeros((Dh * j, _TQ), bf16))
        parts.append(qh)
        if j < 3:
            parts.append(jnp.zeros((128 - Dh * (j + 1), _TQ), bf16))
        return jnp.concatenate(parts, axis=0)

    def step(nqb, ng, nj, s_n, m_n, qb, g, j, s_c, m_c):
        w = qk_weights(nqb, ng, nj)
        hrow = pl.multiple_of(g * 128 + j * Dh, Dh)
        kcol = pl.ds(pl.multiple_of(ng * 128, 128), 128)
        m_run = None
        l = o = None
        for c in range(_NSUB):
            s = jnp.dot(k_s[c * KC:(c + 1) * KC, kcol], w,
                        preferred_element_type=f32)
            s_n[c * KC:(c + 1) * KC, :] = s
            mm = jnp.max(s.reshape(KC // 8, 8, _TQ), axis=0)
            m_run = mm if m_run is None else jnp.maximum(m_run, mm)

            ct, pc = c // kp, c % kp
            cols = slice(ct * 128, (ct + 1) * 128)
            rws = slice(pc * KP, (pc + 1) * KP)
            p = jnp.exp2(s_c[rws, cols].reshape(KP // 8, 8, 128)
                         - m_c[:, cols][None])
            ll = jnp.sum(p, axis=0)
            oo = jnp.dot(vt_s[pl.ds(hrow, Dh), rws],
                         p.reshape(KP, 128).astype(bf16),
                         preferred_element_type=f32)
            l, o = (ll, oo) if pc == 0 else (l + ll, o + oo)
            if pc == kp - 1:
                ls = jnp.sum(l, axis=0, keepdims=True)
                ot_s[pl.ds(hrow, Dh),
                     pl.ds(pl.multiple_of(qb * _TQ + ct * 128, 128), 128)] = (
                         o / ls)
        m_n[...] = jnp.broadcast_to(
            jnp.max(m_run, axis=0, keepdims=True), (8, _TQ))

    s0 = jnp.dot(k_s[:, 0:128], qk_weights(0, 0, 0), preferred_element_type=f32)
    s_a[...] = s0
    m_a[...] = jnp.broadcast_to(jnp.max(s0, axis=0, keepdims=True), (8, _TQ))

    def phase2(u, carry):
        qb = u // _H
        g = (u % _H) // 4
        un = jnp.minimum(u + 1, NU - 1)
        nqb = un // _H
        ng = (un % _H) // 4
        for j in range(4):
            @pl.when(u % 4 == j)
            def _():
                if j % 2 == 0:
                    step(nqb, ng, (j + 1) % 4, s_b, m_b, qb, g, j, s_a, m_a)
                else:
                    step(nqb, ng, (j + 1) % 4, s_a, m_a, qb, g, j, s_b, m_b)
        return carry

    lax.fori_loop(0, NU, phase2, 0)

    wo_copy.wait()
    w1_copy.wait()
    w2_copy.wait()
    b1_copy.wait()
    b2_copy.wait()

    def out_copy(i):
        return pltpu.make_async_copy(
            out_v.at[i % 2], out_hbm.at[0, pl.ds(i * _TM3, _TM3), :],
            sem_o.at[i % 2])

    def phase3(i, carry):
        r0 = pl.multiple_of(i * _TM3, _TM3)
        rows = pl.ds(r0, _TM3)
        o = ot_s[:, rows].T.astype(bf16)
        h = x_v[rows, :].astype(f32) + jnp.dot(
            o, wo_v[...], preferred_element_type=f32)
        y = _layernorm(_layernorm(h)).astype(bf16)
        for c in range(F // _FC):
            cs = slice(c * _FC, (c + 1) * _FC)
            a = jnp.dot(y, w1_v[:, cs], preferred_element_type=f32)
            a = a + b1_v[:, cs].astype(f32)
            g_s[:, cs] = jax.nn.gelu(a, approximate=True).astype(bf16)
        r = jnp.dot(g_s[...], w2_v[...], preferred_element_type=f32)
        res = h + (r + b2_v[...].astype(f32))

        @pl.when(i >= 2)
        def _():
            out_copy(i - 2).wait()

        out_v[i % 2] = res.astype(bf16)
        out_copy(i).start()
        return carry

    lax.fori_loop(0, n3, phase3, 0)
    for i in range(max(n3 - 2, 0), n3):
        out_copy(i).wait()


@jax.jit
def pallas_sequential_preLN__softmax_full_mha__mixer_channel_mlp__prompt_kernel(
    A_x: jax.Array,
    A_wqkv: jax.Array,
    A_wo: jax.Array,
    B_x: jax.Array,
    B_w1: jax.Array,
    B_b1: jax.Array,
    B_w2: jax.Array,
    B_b2: jax.Array,
):
    del B_x
    B, S, D = A_x.shape
    F = B_w1.shape[1]
    assert B == 1
    f32, bf16 = jnp.float32, jnp.bfloat16

    any_spec = pl.BlockSpec(memory_space=pl.ANY)
    scratch = [
        pltpu.VMEM((S, D), bf16),
        pltpu.VMEM((D, 3 * D), bf16),
        pltpu.VMEM((D, D), bf16),
        pltpu.VMEM((D, F), bf16),
        pltpu.VMEM((1, F), bf16),
        pltpu.VMEM((F, D), bf16),
        pltpu.VMEM((1, D), bf16),
        pltpu.VMEM((D, S), bf16),
        pltpu.VMEM((S, D), bf16),
        pltpu.VMEM((D, S), bf16),
        pltpu.VMEM((D, S), f32),
        pltpu.VMEM((S, _TQ), f32),
        pltpu.VMEM((S, _TQ), f32),
        pltpu.VMEM((8, _TQ), f32),
        pltpu.VMEM((8, _TQ), f32),
        pltpu.VMEM((_TM3, F), bf16),
        pltpu.VMEM((2, _TM3, D), bf16),
        pltpu.SemaphoreType.DMA((S // _TM1,)),
        pltpu.SemaphoreType.DMA((8,)),
        pltpu.SemaphoreType.DMA((2,)),
    ]
    return pl.pallas_call(
        functools.partial(_kernel, S=S, D=D, F=F),
        out_shape=jax.ShapeDtypeStruct((B, S, D), bf16),
        in_specs=[any_spec] * 7,
        out_specs=any_spec,
        scratch_shapes=scratch,
        compiler_params=pltpu.CompilerParams(
            vmem_limit_bytes=120 * 1024 * 1024),
    )(A_x, A_wqkv, A_wo, B_w1, B_b1.reshape(1, F), B_w2, B_b2.reshape(1, D))
```

```python
import functools
import math

import jax
import jax.numpy as jnp
from jax import lax
import jax.experimental.pallas as pl
import jax.experimental.pallas.tpu as pltpu

_EPS = 1e-5
_H = 32
_TM1 = 512
_CW = 768
_XP = 128
_TM3 = 128
_FC = 512
_QKC = 512
_KP = 512
_SPAD = 136
_SCOPES = False


def _layernorm(x):
    m = jnp.mean(x, axis=-1, keepdims=True)
    xc = x - m
    v = jnp.mean(xc * xc, axis=-1, keepdims=True)
    return xc * lax.rsqrt(v + _EPS)


class _NullCtx:
    def __enter__(self):
        return self

    def __exit__(self, *a):
        return False


def _scope(name):
    return jax.named_scope(name) if _SCOPES else _NullCtx()


def _kernel(x_hbm, wqkv_hbm, wo_hbm, w1_hbm, b1_hbm, w2_hbm, b2_hbm, out_hbm,
            x_v, wqkv_v, wo_v, w1_v, b1_v, w2_v, b2_v,
            y1_s, qvt_s, k_s, ot_s, s_a, s_b, m_a, m_b, h_s, y3_s, out_v,
            sem_x, sem_w, sem_o, *, S, D, F):
    f32, bf16 = jnp.float32, jnp.bfloat16
    Dh = D // _H
    nxp = S // _XP
    ppb = _TM1 // _XP
    ncw = 3 * D // _CW
    assert ncw == ppb
    n3 = S // _TM3
    dt = D // 128

    def x_copy(i):
        r0 = i * _XP
        if not isinstance(i, int):
            r0 = pl.multiple_of(r0, _XP)
        return pltpu.make_async_copy(
            x_hbm.at[0, pl.ds(r0, _XP), :], x_v.at[pl.ds(r0, _XP), :],
            sem_x.at[i])

    def wqkv_copy(c):
        c0 = c * _CW
        if not isinstance(c, int):
            c0 = pl.multiple_of(c0, 128)
        return pltpu.make_async_copy(
            wqkv_hbm.at[:, pl.ds(c0, _CW)], wqkv_v.at[:, pl.ds(c0, _CW)],
            sem_w.at[c])

    late_copies = [
        pltpu.make_async_copy(wo_hbm, wo_v, sem_w.at[ncw]),
        pltpu.make_async_copy(w1_hbm, w1_v, sem_w.at[ncw + 1]),
        pltpu.make_async_copy(w2_hbm, w2_v, sem_w.at[ncw + 2]),
        pltpu.make_async_copy(b1_hbm, b1_v, sem_w.at[ncw + 3]),
        pltpu.make_async_copy(b2_hbm, b2_v, sem_w.at[ncw + 4]),
    ]

    for i in range(ppb):
        x_copy(i).start()
    wqkv_copy(0).start()
    x_copy(ppb).start()
    wqkv_copy(1).start()
    x_copy(ppb + 1).start()

    qscale = (Dh ** -0.5) * math.log2(math.e)

    def ln1(p):
        r0 = p * _XP
        if not isinstance(p, int):
            r0 = pl.multiple_of(r0, _XP)
        rows = pl.ds(r0, _XP)
        y1_s[rows, :] = _layernorm(x_v[rows, :].astype(f32)).astype(bf16)

    def ln1_first(p, carry):
        x_copy(p).wait()
        ln1(p)
        return carry

    def phase1(t, carry):
        i = t // ncw
        c = t % ncw

        @pl.when(t + 2 < ncw)
        def _():
            wqkv_copy(t + 2).start()

        @pl.when(t + ppb + 2 < nxp)
        def _():
            x_copy(t + ppb + 2).start()

        @pl.when(t < ncw)
        def _():
            wqkv_copy(t).wait()

        @pl.when(t + ppb < nxp)
        def _():
            x_copy(t + ppb).wait()

        rows = pl.ds(pl.multiple_of(i * _TM1, _TM1), _TM1)
        c0 = pl.multiple_of(c * _CW, 128)
        res = jnp.dot(y1_s[rows, :], wqkv_v[:, pl.ds(c0, _CW)],
                      preferred_element_type=f32)
        for j in range(_CW // 128):
            g = c * (_CW // 128) + j
            r = res[:, j * 128:(j + 1) * 128] * jnp.where(g < dt, qscale, 1.0)
            is_k = jnp.logical_and(g >= dt, g < 2 * dt)
            kt = jnp.where(is_k, g - dt, dt)
            tt = jnp.where(is_k, 2 * dt, jnp.where(g < dt, g, g - dt))
            k_s[rows, pl.ds(pl.multiple_of(kt * 128, 128), 128)] = (
                r.astype(bf16))
            qvt_s[pl.ds(pl.multiple_of(tt * 128, 128), 128), rows] = (
                r.T.astype(bf16))
        ln1(jnp.minimum(t + ppb, nxp - 1))
        return carry

    with _scope("phase1"):
        lax.fori_loop(0, ppb, ln1_first, 0)
        lax.fori_loop(0, (S // _TM1) * ncw, phase1, 0)

    for c in late_copies:
        c.start()

    def head_rows(h, base):
        r0 = base + h * Dh
        if not isinstance(h, int):
            r0 = pl.multiple_of(r0, Dh)
        return pl.ds(r0, Dh)

    def qk_weights(h, c0):
        qh = qvt_s[head_rows(h, 0), pl.ds(c0, _QKC)]
        z = jnp.zeros_like(qh)
        j = h % 4
        return jnp.concatenate(
            [jnp.where(j == b, qh, z) for b in range(4)], axis=0)

    nkb = S // 128
    npc = S // _KP
    tpc = _QKC // 128

    def make_qk(h, s_n, m_n):
        st = {}
        k0 = (h // 4) * 128
        if not isinstance(h, int):
            k0 = pl.multiple_of(k0, 128)
        kcols = pl.ds(k0, 128)

        def qk(cb, kb):
            c0 = cb * _QKC
            if not isinstance(cb, int):
                c0 = pl.multiple_of(c0, _QKC)
            if kb == 0:
                st['w'] = qk_weights(h, c0)
            s = jnp.dot(k_s[kb * 128:(kb + 1) * 128, kcols], st['w'],
                        preferred_element_type=f32)
            for t in range(tpc):
                s_n[cb * tpc + t, kb, 0:128, :] = s[:, t * 128:(t + 1) * 128]
            mm = jnp.max(s.reshape(16, 8, _QKC), axis=0)
            st['m'] = mm if kb == 0 else jnp.maximum(st['m'], mm)
            if kb == nkb - 1:
                m_n[:, pl.ds(c0, _QKC)] = jnp.broadcast_to(
                    jnp.max(st['m'], axis=0, keepdims=True), (8, _QKC))
        return qk

    def make_sm(h, s_c, m_c):
        st = {}
        ktp = _KP // 128

        def sm(ct, pc):
            cols = slice(ct * 128, (ct + 1) * 128)
            p = jnp.exp2(
                s_c[ct, pc * ktp:(pc + 1) * ktp, 0:128, :].reshape(
                    _KP // 8, 8, 128) - m_c[:, cols][None])
            for t in range(ktp):
                for r in reversed(range(8)):
                    pair = p[t * 16 + 2 * r] + p[t * 16 + 2 * r + 1]
                    first = pc == 0 and r == 7
                    st['l', t] = pair if first else st['l', t] + pair
            o = jnp.dot(qvt_s[head_rows(h, D), pc * _KP:(pc + 1) * _KP],
                        p.reshape(_KP, 128).astype(bf16),
                        preferred_element_type=f32)
            st['o'] = o if pc == 0 else o + st['o']
            if pc == npc - 1:
                l = st['l', 0]
                for t in range(1, ktp):
                    l = l + st['l', t]
                ot_s[head_rows(h, 0), cols] = (
                    st['o'] / jnp.sum(l, axis=0, keepdims=True))
        return sm

    def step(h, s_c, m_c, s_n, m_n):
        qk = make_qk(h + 1, s_n, m_n)
        sm = make_sm(h, s_c, m_c)
        qk_ids = [(cb, kb) for cb in range(S // _QKC) for kb in range(nkb)]
        sm_ids = [(ct, pc) for ct in range(S // 128) for pc in range(npc)]
        assert len(qk_ids) == len(sm_ids)
        for a, b in zip(qk_ids, sm_ids):
            qk(*a)
            sm(*b)

    def prologue(cb, carry):
        qk = make_qk(0, s_a, m_a)
        for kb in range(nkb):
            qk(cb, kb)
        return carry

    def phase2(h, carry):
        @pl.when(h % 2 == 0)
        def _():
            step(h, s_a, m_a, s_b, m_b)

        @pl.when(h % 2 == 1)
        def _():
            step(h, s_b, m_b, s_a, m_a)
        return carry

    with _scope("attn_pro"):
        lax.fori_loop(0, S // _QKC, prologue, 0)
    with _scope("phase2"):
        lax.fori_loop(0, _H - 1, phase2, 0)

    for c in late_copies:
        c.wait()

    def out_copy(i):
        r0 = i * _TM3
        if not isinstance(i, int):
            r0 = pl.multiple_of(r0, _TM3)
        return pltpu.make_async_copy(
            out_v.at[i % 2], out_hbm.at[0, pl.ds(r0, _TM3), :],
            sem_o.at[i % 2])

    def stage_a_pieces(i):
        r0 = i * _TM3
        if not isinstance(i, int):
            r0 = pl.multiple_of(r0, _TM3)
        rows = pl.ds(r0, _TM3)
        st = {'h': []}

        def proj(n):
            if n == 0:
                st['o'] = ot_s[:, rows].T.astype(bf16)
            cs = slice(n * 128, (n + 1) * 128)
            st['h'].append(x_v[rows, cs].astype(f32) + jnp.dot(
                st['o'], wo_v[:, cs], preferred_element_type=f32))

        def norm():
            h = jnp.concatenate(st['h'], axis=1)
            h_s[i % 2] = h
            y3_s[...] = _layernorm(_layernorm(h)).astype(bf16)

        return [functools.partial(proj, n) for n in range(dt)] + [norm]

    with _scope("attn_epi"):
        sm_last = make_sm(_H - 1, s_b, m_b)
        pieces = stage_a_pieces(0)
        first_ct = _TM3 // 128
        for ct in range(S // 128):
            for pc in range(npc):
                sm_last(ct, pc)
            if ct >= first_ct and pieces:
                pieces.pop(0)()
        assert not pieces

    def phase3(i, carry):
        @pl.when(i >= 2)
        def _():
            out_copy(i - 2).wait()

        y = y3_s[...]
        gs = []
        for c in range(F // _FC):
            a = jnp.dot(y, w1_v[:, c * _FC:(c + 1) * _FC],
                        preferred_element_type=f32)
            a = a + b1_v[pl.ds(c * _FC, _FC)].astype(f32).reshape(1, _FC)
            gs.append(jax.nn.gelu(a, approximate=True).astype(bf16))
        nxt = jnp.minimum(i + 1, n3 - 1)
        stage_next(nxt, i)
        g = jnp.concatenate(gs, axis=1)
        r = jnp.dot(g, w2_v[...], preferred_element_type=f32)
        res = h_s[i % 2] + (r + b2_v[...].astype(f32).reshape(1, D))
        out_v[i % 2] = res.astype(bf16)
        out_copy(i).start()
        return carry

    def stage_next(nxt, i):
        rows = pl.ds(pl.multiple_of(nxt * _TM3, _TM3), _TM3)
        o = ot_s[:, rows].T.astype(bf16)
        h = x_v[rows, :].astype(f32) + jnp.dot(
            o, wo_v[...], preferred_element_type=f32)
        h_s[(i + 1) % 2] = h
        y3_s[...] = _layernorm(_layernorm(h)).astype(bf16)

    with _scope("phase3"):
        lax.fori_loop(0, n3, phase3, 0)
        for i in range(max(n3 - 2, 0), n3):
            out_copy(i).wait()


@jax.jit
def pallas_sequential_preLN__softmax_full_mha__mixer_channel_mlp__prompt_kernel(
    A_x: jax.Array,
    A_wqkv: jax.Array,
    A_wo: jax.Array,
    B_x: jax.Array,
    B_w1: jax.Array,
    B_b1: jax.Array,
    B_w2: jax.Array,
    B_b2: jax.Array,
):
    del B_x
    B, S, D = A_x.shape
    F = B_w1.shape[1]
    assert B == 1
    f32, bf16 = jnp.float32, jnp.bfloat16

    any_spec = pl.BlockSpec(memory_space=pl.ANY)
    s_shape = (S // 128, S // 128, _SPAD, 128)
    scratch = [
        pltpu.VMEM((S, D), bf16),
        pltpu.VMEM((D, 3 * D), bf16),
        pltpu.VMEM((D, D), bf16),
        pltpu.VMEM((D, F), bf16),
        pltpu.VMEM((F,), bf16),
        pltpu.VMEM((F, D), bf16),
        pltpu.VMEM((D,), bf16),
        pltpu.VMEM((S, D), bf16),
        pltpu.VMEM((2 * D + 128, S), bf16),
        pltpu.VMEM((S, D + 128), bf16),
        pltpu.VMEM((D, S), f32),
        pltpu.VMEM(s_shape, f32),
        pltpu.VMEM(s_shape, f32),
        pltpu.VMEM((8, S), f32),
        pltpu.VMEM((8, S), f32),
        pltpu.VMEM((2, _TM3, D), f32),
        pltpu.VMEM((_TM3, D), bf16),
        pltpu.VMEM((2, _TM3, D), bf16),
        pltpu.SemaphoreType.DMA((S // _XP,)),
        pltpu.SemaphoreType.DMA((3 * D // _CW + 5,)),
        pltpu.SemaphoreType.DMA((2,)),
    ]
    return pl.pallas_call(
        functools.partial(_kernel, S=S, D=D, F=F),
        out_shape=jax.ShapeDtypeStruct((B, S, D), bf16),
        in_specs=[any_spec] * 7,
        out_specs=any_spec,
        scratch_shapes=scratch,
        compiler_params=pltpu.CompilerParams(
            vmem_limit_bytes=120 * 1024 * 1024),
    )(A_x, A_wqkv, A_wo, B_w1, B_b1, B_w2, B_b2)
```

```python
import functools
import math

import jax
import jax.numpy as jnp
from jax import lax
import jax.experimental.pallas as pl
import jax.experimental.pallas.tpu as pltpu

_EPS = 1e-5
_H = 32
_TM1 = 512
_CW = 768
_XP = 128
_TM3 = 128
_FC = 512
_QKC = 512
_KP = 512
_SPAD = 136
_EPI_EVERY = 3
_SCOPES = False


def _layernorm(x):
    m = jnp.mean(x, axis=-1, keepdims=True)
    xc = x - m
    v = jnp.mean(xc * xc, axis=-1, keepdims=True)
    return xc * lax.rsqrt(v + _EPS)


def _pack(x):
    return pltpu.bitcast(x, jnp.uint32)


def _unpack(x):
    return pltpu.bitcast(x, jnp.bfloat16)


def _ds(start, size, align):
    if not isinstance(start, int):
        start = pl.multiple_of(start, align)
    return pl.ds(start, size)


class _NullCtx:
    def __enter__(self):
        return self

    def __exit__(self, *a):
        return False


def _scope(name):
    return jax.named_scope(name) if _SCOPES else _NullCtx()


def _kernel(x_hbm, wqkv_hbm, wo_hbm, w1_hbm, b1_hbm, w2_hbm, b2_hbm, out_hbm,
            x_v, wqkv_v, wo_v, w1_v, b1_v, w2_v, b2_v,
            y1_s, nat_s, qvt_s, ot_s, s_a, s_b, m_a, m_b,
            kc_a, kc_b, qc_a, qc_b, vc_a, vc_b, h_s, y3_s, out_v,
            sem_x, sem_w, sem_o, *, S, D, F):
    f32, bf16 = jnp.float32, jnp.bfloat16
    Dh = D // _H
    nxp = S // _XP
    ppb = _TM1 // _XP
    ncw = 3 * D // _CW
    assert ncw == ppb
    n1 = (S // _TM1) * ncw
    n3 = S // _TM3
    dt = D // 128
    tpw = _CW // 128

    def x_copy(i):
        rows = _ds(i * _XP, _XP, _XP)
        return pltpu.make_async_copy(
            x_hbm.at[0, rows, :], x_v.at[rows, :], sem_x.at[i])

    def wqkv_copy(c):
        cols = _ds(c * _CW, _CW, 128)
        return pltpu.make_async_copy(
            wqkv_hbm.at[:, cols], wqkv_v.at[:, cols], sem_w.at[c])

    late_copies = [
        pltpu.make_async_copy(wo_hbm, wo_v, sem_w.at[ncw]),
        pltpu.make_async_copy(w1_hbm, w1_v, sem_w.at[ncw + 1]),
        pltpu.make_async_copy(w2_hbm, w2_v, sem_w.at[ncw + 2]),
        pltpu.make_async_copy(b1_hbm, b1_v, sem_w.at[ncw + 3]),
        pltpu.make_async_copy(b2_hbm, b2_v, sem_w.at[ncw + 4]),
    ]

    for i in range(ppb):
        x_copy(i).start()
    wqkv_copy(0).start()
    x_copy(ppb).start()
    wqkv_copy(1).start()
    x_copy(ppb + 1).start()

    qscale = (Dh ** -0.5) * math.log2(math.e)

    def ln1(p):
        y = _layernorm(x_v[_ds(p * _XP, _XP, _XP), :].astype(f32))
        y1_s[_ds(p * (_XP // 2), _XP // 2, _XP // 2), :] = _pack(
            y.astype(bf16))

    def ln1_first(p, carry):
        x_copy(p).wait()
        ln1(p)
        return carry

    def transpose_tile(i, g):
        is_k = jnp.logical_and(g >= dt, g < 2 * dt)
        tt = jnp.where(is_k, 2 * dt, jnp.where(g < dt, g, g - dt))
        hrows = _ds(i * (_TM1 // 2), _TM1 // 2, _TM1 // 2)
        r = _unpack(nat_s[hrows, _ds(g * 128, 128, 128)])
        qvt_s[_ds(tt * 64, 64, 64), _ds(i * _TM1, _TM1, _TM1)] = _pack(r.T)

    def phase1(t, carry):
        i = t // ncw
        c = t % ncw

        @pl.when(t + 2 < ncw)
        def _():
            wqkv_copy(t + 2).start()

        @pl.when(t + ppb + 2 < nxp)
        def _():
            x_copy(t + ppb + 2).start()

        @pl.when(t < ncw)
        def _():
            wqkv_copy(t).wait()

        @pl.when(t + ppb < nxp)
        def _():
            x_copy(t + ppb).wait()

        tp = jnp.maximum(t - 1, 0)
        for j in range(tpw):
            transpose_tile(tp // ncw, (tp % ncw) * tpw + j)
        hrows = _ds(i * (_TM1 // 2), _TM1 // 2, _TM1 // 2)
        res = jnp.dot(_unpack(y1_s[hrows, :]), wqkv_v[:, _ds(c * _CW, _CW, 128)],
                      preferred_element_type=f32)
        for j in range(tpw):
            g = c * tpw + j
            r = res[:, j * 128:(j + 1) * 128] * jnp.where(g < dt, qscale, 1.0)
            nat_s[hrows, _ds(g * 128, 128, 128)] = _pack(r.astype(bf16))
        ln1(jnp.minimum(t + ppb, nxp - 1))
        return carry

    with _scope("phase1"):
        nat_s[0:_TM1 // 2, 0:_CW] = jnp.zeros((_TM1 // 2, _CW), jnp.uint32)
        lax.fori_loop(0, ppb, ln1_first, 0)
        lax.fori_loop(0, n1, phase1, 0)

    for c in late_copies:
        c.start()

    nkb = S // 128
    npc = S // _KP
    tpc = _QKC // 128
    hh = Dh // 2

    def stage_piece(n, nn, hq, hv, kc, qc, vc):
        rows = _ds(n * (S // 2 // nn), S // 2 // nn, S // 2 // nn)
        cols = _ds(n * (S // nn), S // nn, S // nn)
        kc[rows, :] = nat_s[rows, _ds(D + (hq // 4) * 128, 128, 128)]
        qh = qvt_s[_ds(hq * hh, hh, hh), cols]
        z = jnp.zeros_like(qh)
        for b in range(4):
            qc[b * hh:(b + 1) * hh, cols] = jnp.where(hq % 4 == b, qh, z)
        vc[:, cols] = qvt_s[_ds(D // 2 + hv * hh, hh, hh), cols]

    def make_qk(k_tile, q_cols, s_n, m_n):
        st = {}

        def qk(cb, kb):
            cols = _ds(cb * _QKC, _QKC, _QKC)
            if kb == 0:
                st['w'] = _unpack(q_cols(cols))
            s = jnp.dot(_unpack(k_tile(kb)), st['w'],
                        preferred_element_type=f32)
            for t in range(tpc):
                s_n[cb * tpc + t, kb, 0:128, :] = s[:, t * 128:(t + 1) * 128]
            mm = jnp.max(s.reshape(16, 8, _QKC), axis=0)
            st['m'] = mm if kb == 0 else jnp.maximum(st['m'], mm)
            if kb == nkb - 1:
                m_n[:, cols] = jnp.broadcast_to(
                    jnp.max(st['m'], axis=0, keepdims=True), (8, _QKC))
        return qk

    def make_sm(h, vc, s_c, m_c):
        st = {}
        ktp = _KP // 128

        def sm(ct, pc):
            cols = slice(ct * 128, (ct + 1) * 128)
            p = jnp.exp2(
                s_c[ct, pc * ktp:(pc + 1) * ktp, 0:128, :].reshape(
                    _KP // 8, 8, 128) - m_c[:, cols][None])
            for t in range(ktp):
                for r in reversed(range(8)):
                    pair = p[t * 16 + 2 * r] + p[t * 16 + 2 * r + 1]
                    first = pc == 0 and r == 7
                    st['l', t] = pair if first else st['l', t] + pair
            o = jnp.dot(_unpack(vc[:, pc * _KP:(pc + 1) * _KP]),
                        p.reshape(_KP, 128).astype(bf16),
                        preferred_element_type=f32)
            st['o'] = o if pc == 0 else o + st['o']
            if pc == npc - 1:
                l = st['l', 0]
                for t in range(1, ktp):
                    l = l + st['l', t]
                ot_s[_ds(h * Dh, Dh, Dh), cols] = (
                    st['o'] / jnp.sum(l, axis=0, keepdims=True))
        return sm

    def step(h, cur, nxt):
        (s_c, m_c, kc, qc, vc), (s_n, m_n, kn, qn, vn) = cur, nxt
        qk = make_qk(lambda kb: kc[kb * 64:(kb + 1) * 64, :],
                     lambda cols: qc[:, cols], s_n, m_n)
        sm = make_sm(h, vc, s_c, m_c)
        qk_ids = [(cb, kb) for cb in range(S // _QKC) for kb in range(nkb)]
        sm_ids = [(ct, pc) for ct in range(S // 128) for pc in range(npc)]
        assert len(qk_ids) == len(sm_ids)
        hq = jnp.minimum(h + 2, _H - 1)
        for n, (a, b) in enumerate(zip(qk_ids, sm_ids)):
            qk(*a)
            sm(*b)
            if n % 3 == 2 and n // 3 < 16:
                stage_piece(n // 3, 16, hq, h + 1, kn, qn, vn)

    buf_a = (s_a, m_a, kc_a, qc_a, vc_a)
    buf_b = (s_b, m_b, kc_b, qc_b, vc_b)

    def prologue(cb, carry):
        def q0(cols):
            qh = qvt_s[0:hh, cols]
            return jnp.concatenate(
                [qh, jnp.zeros((3 * hh, _QKC), jnp.uint32)], axis=0)

        qk = make_qk(lambda kb: nat_s[kb * 64:(kb + 1) * 64, D:D + 128],
                     q0, s_a, m_a)
        g0 = (ncw - 1) * tpw
        for kb in range(nkb):
            qk(cb, kb)
            if kb == 1:
                stage_piece(cb, S // _QKC, 1, 0, kc_a, qc_a, vc_a)
            if kb == 5:
                transpose_tile(S // _TM1 - 1, g0 + cb)
            if kb == 9:
                transpose_tile(S // _TM1 - 1,
                               g0 + jnp.minimum(cb + 4, tpw - 1))
        return carry

    def phase2(h, carry):
        @pl.when(h % 2 == 0)
        def _():
            step(h, buf_a, buf_b)

        @pl.when(h % 2 == 1)
        def _():
            step(h, buf_b, buf_a)
        return carry

    with _scope("attn_pro"):
        lax.fori_loop(0, S // _QKC, prologue, 0)
    with _scope("phase2"):
        lax.fori_loop(0, _H - 1, phase2, 0)

    for c in late_copies:
        c.wait()

    def out_copy(i):
        return pltpu.make_async_copy(
            out_v.at[i % 2], out_hbm.at[0, _ds(i * _TM3, _TM3, _TM3), :],
            sem_o.at[i % 2])

    def stage_a_pieces(i, slot, nsplit, ksplit):
        rows = _ds(i * _TM3, _TM3, _TM3)
        st = {'h': []}
        w = D // nsplit
        kw = D // ksplit

        def proj(n, k):
            if n == 0:
                st['o', k] = ot_s[k * kw:(k + 1) * kw, rows].T.astype(bf16)
            cs = slice(n * w, (n + 1) * w)
            acc = x_v[rows, cs].astype(f32) if k == 0 else st['h'].pop()
            st['h'].append(acc + jnp.dot(
                st['o', k], wo_v[k * kw:(k + 1) * kw, cs],
                preferred_element_type=f32))

        def norm():
            h = jnp.concatenate(st['h'], axis=1)
            h_s[slot] = h
            y3_s[...] = _pack(_layernorm(_layernorm(h)).astype(bf16))

        return [functools.partial(proj, n, k) for n in range(nsplit)
                for k in range(ksplit)] + [norm]

    with _scope("attn_epi"):
        sm_last = make_sm(_H - 1, vc_b, s_b, m_b)
        pieces = stage_a_pieces(0, 0, dt, 2)
        first = (_TM3 // 128) * npc
        for n in range((S // 128) * npc):
            sm_last(n // npc, n % npc)
            if n >= first and (n - first) % _EPI_EVERY == 0 and pieces:
                pieces.pop(0)()
        assert not pieces

    def phase3(i, carry):
        @pl.when(i >= 2)
        def _():
            out_copy(i - 2).wait()

        y = _unpack(y3_s[...])
        gs = []
        for c in range(F // _FC):
            a = jnp.dot(y, w1_v[:, c * _FC:(c + 1) * _FC],
                        preferred_element_type=f32)
            a = a + b1_v[pl.ds(c * _FC, _FC)].astype(f32).reshape(1, _FC)
            gs.append(jax.nn.gelu(a, approximate=True).astype(bf16))
        for piece in stage_a_pieces(jnp.minimum(i + 1, n3 - 1), (i + 1) % 2, 1, 1):
            piece()
        g = jnp.concatenate(gs, axis=1)
        r = jnp.dot(g, w2_v[...], preferred_element_type=f32)
        res = h_s[i % 2] + (r + b2_v[...].astype(f32).reshape(1, D))
        out_v[i % 2] = res.astype(bf16)
        out_copy(i).start()
        return carry

    with _scope("phase3"):
        lax.fori_loop(0, n3, phase3, 0)
        for i in range(max(n3 - 2, 0), n3):
            out_copy(i).wait()


@jax.jit
def pallas_sequential_preLN__softmax_full_mha__mixer_channel_mlp__prompt_kernel(
    A_x: jax.Array,
    A_wqkv: jax.Array,
    A_wo: jax.Array,
    B_x: jax.Array,
    B_w1: jax.Array,
    B_b1: jax.Array,
    B_w2: jax.Array,
    B_b2: jax.Array,
):
    del B_x
    B, S, D = A_x.shape
    F = B_w1.shape[1]
    assert B == 1
    f32, bf16, u32 = jnp.float32, jnp.bfloat16, jnp.uint32
    Dh = D // _H

    any_spec = pl.BlockSpec(memory_space=pl.ANY)
    s_shape = (S // 128, S // 128, _SPAD, 128)
    scratch = [
        pltpu.VMEM((S, D), bf16),
        pltpu.VMEM((D, 3 * D), bf16),
        pltpu.VMEM((D, D), bf16),
        pltpu.VMEM((D, F), bf16),
        pltpu.VMEM((F,), bf16),
        pltpu.VMEM((F, D), bf16),
        pltpu.VMEM((D,), bf16),
        pltpu.VMEM((S // 2, D), u32),
        pltpu.VMEM((S // 2, 3 * D), u32),
        pltpu.VMEM((D + 64, S), u32),
        pltpu.VMEM((D, S), f32),
        pltpu.VMEM(s_shape, f32),
        pltpu.VMEM(s_shape, f32),
        pltpu.VMEM((8, S), f32),
        pltpu.VMEM((8, S), f32),
        pltpu.VMEM((S // 2, 128), u32),
        pltpu.VMEM((S // 2, 128), u32),
        pltpu.VMEM((64, S), u32),
        pltpu.VMEM((64, S), u32),
        pltpu.VMEM((Dh // 2, S), u32),
        pltpu.VMEM((Dh // 2, S), u32),
        pltpu.VMEM((2, _TM3, D), f32),
        pltpu.VMEM((_TM3 // 2, D), u32),
        pltpu.VMEM((2, _TM3, D), bf16),
        pltpu.SemaphoreType.DMA((S // _XP,)),
        pltpu.SemaphoreType.DMA((3 * D // _CW + 5,)),
        pltpu.SemaphoreType.DMA((2,)),
    ]
    return pl.pallas_call(
        functools.partial(_kernel, S=S, D=D, F=F),
        out_shape=jax.ShapeDtypeStruct((B, S, D), bf16),
        in_specs=[any_spec] * 7,
        out_specs=any_spec,
        scratch_shapes=scratch,
        compiler_params=pltpu.CompilerParams(
            vmem_limit_bytes=120 * 1024 * 1024),
    )(A_x, A_wqkv, A_wo, B_w1, B_b1, B_w2, B_b2)
```

```python
import functools
import math

import jax
import jax.numpy as jnp
from jax import lax
import jax.experimental.pallas as pl
import jax.experimental.pallas.tpu as pltpu

_EPS = 1e-5
_H = 32
_TM1 = 512
_CW = 768
_CW0 = 256
_XP = 128
_TM3 = 128
_FC = 512
_QKC = 512
_KP = 512
_SPAD = 136
_EPI_EVERY = 3
_EPI_MS = 1
_WPAD = 128
_SCOPES = False


def _layernorm(x):
    m = jnp.mean(x, axis=-1, keepdims=True)
    xc = x - m
    v = jnp.mean(xc * xc, axis=-1, keepdims=True)
    return xc * lax.rsqrt(v + _EPS)


def _pack(x):
    return pltpu.bitcast(x, jnp.uint32)


def _unpack(x):
    return pltpu.bitcast(x, jnp.bfloat16)


def _ds(start, size, align):
    if not isinstance(start, int):
        start = pl.multiple_of(start, align)
    return pl.ds(start, size)


class _NullCtx:
    def __enter__(self):
        return self

    def __exit__(self, *a):
        return False


def _scope(name):
    return jax.named_scope(name) if _SCOPES else _NullCtx()


def _kernel(x_hbm, wqkv_hbm, wo_hbm, w1_hbm, b1_hbm, w2_hbm, b2_hbm, out_hbm,
            x_v, wqkv_v, wo_v, w1_v, b1_v, w2_v, b2_v,
            y1_s, nat_s, qvt_s, ot_s, s_a, s_b, m_a, m_b,
            kc_a, kc_b, qc_a, qc_b, vc_a, vc_b, h_s, y3_s, out_v,
            sem_x, sem_w, sem_o, *, S, D, F):
    f32, bf16 = jnp.float32, jnp.bfloat16
    Dh = D // _H
    nxp = S // _XP
    ppb = _TM1 // _XP
    ncw = 3 * D // _CW
    assert ncw == ppb
    n1 = (S // _TM1) * ncw
    n3 = S // _TM3
    dt = D // 128
    tpw = _CW // 128

    def x_copy(i):
        rows = _ds(i * _XP, _XP, _XP)
        return pltpu.make_async_copy(
            x_hbm.at[0, rows, :], x_v.at[rows, :], sem_x.at[i])

    def wqkv_copy(c):
        cols = _ds(c * _CW, _CW, 128)
        return pltpu.make_async_copy(
            wqkv_hbm.at[:, cols], wqkv_v.at[:, cols], sem_w.at[c])

    nsub0 = _CW // _CW0

    def w0_copy(j):
        cols = _ds(j * _CW0, _CW0, 128)
        return pltpu.make_async_copy(
            wqkv_hbm.at[:, cols], wqkv_v.at[:, cols], sem_w.at[ncw + 5 + j])

    late_copies = [
        pltpu.make_async_copy(wo_hbm, wo_v, sem_w.at[ncw]),
        pltpu.make_async_copy(w1_hbm, w1_v, sem_w.at[ncw + 1]),
        pltpu.make_async_copy(w2_hbm, w2_v, sem_w.at[ncw + 2]),
        pltpu.make_async_copy(b1_hbm, b1_v, sem_w.at[ncw + 3]),
        pltpu.make_async_copy(b2_hbm, b2_v, sem_w.at[ncw + 4]),
    ]

    for i in range(ppb):
        x_copy(i).start()
    w0_copy(0).start()

    qscale = (Dh ** -0.5) * math.log2(math.e)

    def ln1(p):
        y = _layernorm(x_v[_ds(p * _XP, _XP, _XP), :].astype(f32))
        y1_s[_ds(p * (_XP // 2), _XP // 2, _XP // 2), :] = _pack(
            y.astype(bf16))

    def ln1_first(p, carry):
        x_copy(p).wait()
        ln1(p)
        return carry

    def transpose_tile(i, g):
        is_k = jnp.logical_and(g >= dt, g < 2 * dt)
        tt = jnp.where(is_k, 2 * dt, jnp.where(g < dt, g, g - dt))
        hrows = _ds(i * (_TM1 // 2), _TM1 // 2, _TM1 // 2)
        r = _unpack(nat_s[hrows, _ds(g * 128, 128, 128)])
        qvt_s[_ds(tt * 64, 64, 64), _ds(i * _TM1, _TM1, _TM1)] = _pack(r.T)

    def phase1(t, carry):
        i = t // ncw
        c = t % ncw

        @pl.when(t < ncw)
        def _():
            wqkv_copy(t).wait()

        @pl.when(t + ppb < nxp)
        def _():
            x_copy(t + ppb).wait()

        for j in range(tpw):
            transpose_tile((t - 1) // ncw, ((t - 1) % ncw) * tpw + j)
        hrows = _ds(i * (_TM1 // 2), _TM1 // 2, _TM1 // 2)
        res = jnp.dot(_unpack(y1_s[hrows, :]), wqkv_v[:, _ds(c * _CW, _CW, 128)],
                      preferred_element_type=f32)
        for j in range(tpw):
            g = c * tpw + j
            r = res[:, j * 128:(j + 1) * 128] * jnp.where(g < dt, qscale, 1.0)
            nat_s[hrows, _ds(g * 128, 128, 128)] = _pack(r.astype(bf16))
        ln1(jnp.minimum(t + ppb, nxp - 1))

        @pl.when(t + 2 < ncw)
        def _():
            wqkv_copy(t + 2).start()

        @pl.when(t + ppb + 2 < nxp)
        def _():
            x_copy(t + ppb + 2).start()
        return carry

    def phase1_start(j, carry):
        w0_copy(j).wait()

        @pl.when(j == nsub0 - 1)
        def _():
            x_copy(ppb).wait()

        res = jnp.dot(_unpack(y1_s[0:_TM1 // 2, :]),
                      wqkv_v[:, _ds(j * _CW0, _CW0, 128)],
                      preferred_element_type=f32) * qscale
        nat_s[0:_TM1 // 2, _ds(j * _CW0, _CW0, 128)] = _pack(res.astype(bf16))
        ln1(jnp.where(j == nsub0 - 1, ppb, ppb - 1))

        @pl.when(j == 0)
        def _():
            wqkv_copy(1).start()
            x_copy(ppb + 1).start()

        @pl.when(j == nsub0 - 1)
        def _():
            wqkv_copy(2).start()
            x_copy(ppb + 2).start()
        return carry

    with _scope("phase1"):
        assert _CW <= D
        lax.fori_loop(0, ppb, ln1_first, 0)
        for j in range(1, nsub0):
            w0_copy(j).start()
        x_copy(ppb).start()
        lax.fori_loop(0, nsub0, phase1_start, 0)
        lax.fori_loop(1, n1, phase1, 0)

    for c in late_copies:
        c.start()

    nkb = S // 128
    npc = S // _KP
    tpc = _QKC // 128
    hh = Dh // 2

    def stage_piece(n, nn, hq, hv, kc, qc, vc):
        rows = _ds(n * (S // 2 // nn), S // 2 // nn, S // 2 // nn)
        cols = _ds(n * (S // nn), S // nn, S // nn)
        kc[rows, :] = nat_s[rows, _ds(D + (hq // 4) * 128, 128, 128)]
        qh = qvt_s[_ds(hq * hh, hh, hh), cols]
        z = jnp.zeros_like(qh)
        for b in range(4):
            qc[b * hh:(b + 1) * hh, cols] = jnp.where(hq % 4 == b, qh, z)
        vc[:, cols] = qvt_s[_ds(D // 2 + hv * hh, hh, hh), cols]

    def make_qk(k_tile, q_cols, s_n, m_n):
        st = {}

        def qk(cb, kb):
            cols = _ds(cb * _QKC, _QKC, _QKC)
            if kb == 0:
                st['w'] = _unpack(q_cols(cols))
            s = jnp.dot(_unpack(k_tile(kb)), st['w'],
                        preferred_element_type=f32)
            for t in range(tpc):
                s_n[cb * tpc + t, kb, 0:128, :] = s[:, t * 128:(t + 1) * 128]
            mm = jnp.max(s.reshape(16, 8, _QKC), axis=0)
            st['m'] = mm if kb == 0 else jnp.maximum(st['m'], mm)
            if kb == nkb - 1:
                m_n[:, cols] = jnp.broadcast_to(
                    jnp.max(st['m'], axis=0, keepdims=True), (8, _QKC))
        return qk

    def make_sm(h, vc, s_c, m_c):
        st = {}
        ktp = _KP // 128

        def sm(ct, pc):
            cols = _ds(ct * 128, 128, 128)
            p = jnp.exp2(
                s_c[ct, pc * ktp:(pc + 1) * ktp, 0:128, :].reshape(
                    _KP // 8, 8, 128) - m_c[:, cols][None])
            for t in range(ktp):
                for r in reversed(range(8)):
                    pair = p[t * 16 + 2 * r] + p[t * 16 + 2 * r + 1]
                    first = pc == 0 and r == 7
                    st['l', t] = pair if first else st['l', t] + pair
            o = jnp.dot(_unpack(vc[:, pc * _KP:(pc + 1) * _KP]),
                        p.reshape(_KP, 128).astype(bf16),
                        preferred_element_type=f32)
            st['o'] = o if pc == 0 else o + st['o']
            if pc == npc - 1:
                l = st['l', 0]
                for t in range(1, ktp):
                    l = l + st['l', t]
                ot_s[_ds(h * Dh, Dh, Dh), cols] = (
                    st['o'] / jnp.sum(l, axis=0, keepdims=True))
        return sm

    def step(h, cur, nxt):
        (s_c, m_c, kc, qc, vc), (s_n, m_n, kn, qn, vn) = cur, nxt
        qk = make_qk(lambda kb: kc[kb * 64:(kb + 1) * 64, :],
                     lambda cols: qc[:, cols], s_n, m_n)
        sm = make_sm(h, vc, s_c, m_c)
        qk_ids = [(cb, kb) for cb in range(S // _QKC) for kb in range(nkb)]
        sm_ids = [(ct, pc) for ct in range(S // 128) for pc in range(npc)]
        assert len(qk_ids) == len(sm_ids)
        hq = jnp.minimum(h + 2, _H - 1)
        for n, (a, b) in enumerate(zip(qk_ids, sm_ids)):
            qk(*a)
            sm(*b)
            if n % 3 == 2 and n // 3 < 16:
                stage_piece(n // 3, 16, hq, h + 1, kn, qn, vn)

    buf_a = (s_a, m_a, kc_a, qc_a, vc_a)
    buf_b = (s_b, m_b, kc_b, qc_b, vc_b)

    def prologue(cb, carry):
        def q0(cols):
            qh = qvt_s[0:hh, cols]
            return jnp.concatenate(
                [qh, jnp.zeros((3 * hh, _QKC), jnp.uint32)], axis=0)

        qk = make_qk(lambda kb: nat_s[kb * 64:(kb + 1) * 64, D:D + 128],
                     q0, s_a, m_a)
        g0 = (ncw - 1) * tpw
        for kb in range(nkb):
            qk(cb, kb)
            if kb == 1:
                stage_piece(cb, S // _QKC, 1, 0, kc_a, qc_a, vc_a)
            if kb == 5:
                transpose_tile(S // _TM1 - 1, g0 + cb)
            if kb == 9:
                transpose_tile(S // _TM1 - 1,
                               g0 + jnp.minimum(cb + 4, tpw - 1))
        return carry

    def phase2(h, carry):
        @pl.when(h % 2 == 0)
        def _():
            step(h, buf_a, buf_b)

        @pl.when(h % 2 == 1)
        def _():
            step(h, buf_b, buf_a)
        return carry

    with _scope("attn_pro"):
        lax.fori_loop(0, S // _QKC, prologue, 0)
    with _scope("phase2"):
        lax.fori_loop(0, _H - 1, phase2, 0)

    for c in late_copies:
        c.wait()

    def out_copy(i):
        return pltpu.make_async_copy(
            out_v.at[i % 2], out_hbm.at[0, _ds(i * _TM3, _TM3, _TM3), :],
            sem_o.at[i % 2])

    def stage_a_pieces(i, slot, nsplit, ksplit, msplit=1):
        rows = _ds(i * _TM3, _TM3, _TM3)
        st = {}
        w = D // nsplit
        kw = D // ksplit
        mw = _TM3 // msplit

        def proj(n, k, m):
            if n == 0 and m == 0:
                st['o', k] = ot_s[k * kw:(k + 1) * kw, rows].T.astype(bf16)
            cs = slice(n * w, (n + 1) * w)
            ms = slice(m * mw, (m + 1) * mw)
            if k == 0:
                acc = x_v[_ds(i * _TM3 + m * mw, mw, mw), cs].astype(f32)
            else:
                acc = st['h', n, m]
            st['h', n, m] = acc + jnp.dot(
                st['o', k][ms], wo_v[k * kw:(k + 1) * kw, cs],
                preferred_element_type=f32)

        def norm():
            h = jnp.concatenate(
                [jnp.concatenate([st['h', n, m] for m in range(msplit)], axis=0)
                 for n in range(nsplit)], axis=1)
            h_s[slot] = h
            y3_s[...] = _pack(_layernorm(_layernorm(h)).astype(bf16))

        return [functools.partial(proj, n, k, m) for n in range(nsplit)
                for k in range(ksplit) for m in range(msplit)] + [norm]

    assert _TM3 == 128
    sm_last = make_sm(_H - 1, vc_b, s_b, m_b)

    with _scope("attn_epi"):
        pieces = stage_a_pieces(0, 0, dt, 2)
        for pc in range(npc):
            sm_last(0, pc)
        for n, piece in enumerate(pieces):
            piece()
            if n % 2 == 1 and n // 2 < npc:
                sm_last(1, n // 2)

    def phase3(i, carry):
        @pl.when(i >= 2)
        def _():
            out_copy(i - 2).wait()

        y = _unpack(y3_s[...])
        gs = []
        for c in range(F // _FC):
            a = jnp.dot(y, w1_v[:, c * _FC:(c + 1) * _FC],
                        preferred_element_type=f32)
            a = a + b1_v[pl.ds(c * _FC, _FC)].astype(f32).reshape(1, _FC)
            gs.append(jax.nn.gelu(a, approximate=True).astype(bf16))
            if 1 <= c <= npc:
                sm_last(jnp.minimum(i + 2, n3 - 1), c - 1)
        for piece in stage_a_pieces(i + 1, (i + 1) % 2, 1, 1):
            piece()
        g = jnp.concatenate(gs, axis=1)
        r = jnp.dot(g, w2_v[...], preferred_element_type=f32)
        res = h_s[i % 2] + (r + b2_v[...].astype(f32).reshape(1, D))
        out_v[i % 2] = res.astype(bf16)
        out_copy(i).start()
        return carry

    def last_half(k, carry):
        slot = (n3 - 1) % 2
        fh = F // 2
        y = _unpack(y3_s[...])
        gs = []
        for c0 in range(0, fh, _FC):
            w = min(_FC, fh - c0)
            cs = _ds(k * fh + c0, w, 256)
            a = jnp.dot(y, w1_v[:, cs], preferred_element_type=f32)
            a = a + b1_v[cs].astype(f32).reshape(1, w)
            gs.append(jax.nn.gelu(a, approximate=True).astype(bf16))
        g = jnp.concatenate(gs, axis=1)
        r = h_s[slot] + jnp.dot(g, w2_v[_ds(k * fh, fh, 256), :],
                                preferred_element_type=f32)
        h_s[slot] = r
        out_v[slot] = (r + b2_v[...].astype(f32).reshape(1, D)).astype(bf16)
        return carry

    with _scope("phase3"):
        lax.fori_loop(0, n3 - 1, phase3, 0)
        out_copy(n3 - 3).wait()
        lax.fori_loop(0, 2, last_half, 0)
        out_copy(n3 - 1).start()
        out_copy(n3 - 2).wait()
        out_copy(n3 - 1).wait()


@jax.jit
def pallas_sequential_preLN__softmax_full_mha__mixer_channel_mlp__prompt_kernel(
    A_x: jax.Array,
    A_wqkv: jax.Array,
    A_wo: jax.Array,
    B_x: jax.Array,
    B_w1: jax.Array,
    B_b1: jax.Array,
    B_w2: jax.Array,
    B_b2: jax.Array,
):
    del B_x
    B, S, D = A_x.shape
    F = B_w1.shape[1]
    assert B == 1
    f32, bf16, u32 = jnp.float32, jnp.bfloat16, jnp.uint32
    Dh = D // _H

    any_spec = pl.BlockSpec(memory_space=pl.ANY)
    s_shape = (S // 128, S // 128, _SPAD, 128)
    scratch = [
        pltpu.VMEM((S, D), bf16),
        pltpu.VMEM((D, 3 * D + _WPAD), bf16),
        pltpu.VMEM((D, D), bf16),
        pltpu.VMEM((D, F), bf16),
        pltpu.VMEM((F,), bf16),
        pltpu.VMEM((F, D), bf16),
        pltpu.VMEM((D,), bf16),
        pltpu.VMEM((S // 2, D), u32),
        pltpu.VMEM((S // 2, 3 * D), u32),
        pltpu.VMEM((D + 64, S), u32),
        pltpu.VMEM((D, S), f32),
        pltpu.VMEM(s_shape, f32),
        pltpu.VMEM(s_shape, f32),
        pltpu.VMEM((8, S), f32),
        pltpu.VMEM((8, S), f32),
        pltpu.VMEM((S // 2, 128), u32),
        pltpu.VMEM((S // 2, 128), u32),
        pltpu.VMEM((64, S), u32),
        pltpu.VMEM((64, S), u32),
        pltpu.VMEM((Dh // 2, S), u32),
        pltpu.VMEM((Dh // 2, S), u32),
        pltpu.VMEM((2, _TM3, D), f32),
        pltpu.VMEM((_TM3 // 2, D), u32),
        pltpu.VMEM((2, _TM3, D), bf16),
        pltpu.SemaphoreType.DMA((S // _XP,)),
        pltpu.SemaphoreType.DMA((3 * D // _CW + 5 + _CW // _CW0,)),
        pltpu.SemaphoreType.DMA((2,)),
    ]
    return pl.pallas_call(
        functools.partial(_kernel, S=S, D=D, F=F),
        out_shape=jax.ShapeDtypeStruct((B, S, D), bf16),
        in_specs=[any_spec] * 7,
        out_specs=any_spec,
        scratch_shapes=scratch,
        compiler_params=pltpu.CompilerParams(
            vmem_limit_bytes=120 * 1024 * 1024),
    )(A_x, A_wqkv, A_wo, B_w1, B_b1, B_w2, B_b2)
```

```python
import functools
import math

import jax
import jax.numpy as jnp
from jax import lax
import jax.experimental.pallas as pl
import jax.experimental.pallas.tpu as pltpu

_EPS = 1e-5
_H = 32
_TM1 = 512
_CW = 768
_CW0 = 256
_XP = 128
_TM3 = 128
_FC = 512
_QKC = 512
_KP = 512
_WPAD = 128


def _layernorm(x):
    m = jnp.mean(x, axis=-1, keepdims=True)
    xc = x - m
    v = jnp.mean(xc * xc, axis=-1, keepdims=True)
    return xc * lax.rsqrt(v + _EPS)


def _pack(x):
    return pltpu.bitcast(x, jnp.uint32)


def _unpack(x):
    return pltpu.bitcast(x, jnp.bfloat16)


def _ds(start, size, align):
    if not isinstance(start, int):
        start = pl.multiple_of(start, align)
    return pl.ds(start, size)


def _kernel(x_hbm, wqkv_hbm, wo_hbm, w1_hbm, b1_hbm, w2_hbm, b2_hbm, out_hbm,
            x_v, wqkv_v, wo_v, w1_v, b1_v, w2_v, b2_v,
            y1_s, nat_s, qvt_s, ot_s, s_a, s_b, m_a, m_b,
            kc_a, kc_b, qc_a, qc_b, vc_a, vc_b, h_s, y3_s, out_v,
            sem_x, sem_w, sem_o, *, S, D, F):
    f32, bf16 = jnp.float32, jnp.bfloat16
    Dh = D // _H
    nxp = S // _XP
    ppb = _TM1 // _XP
    ncw = 3 * D // _CW
    nsub0 = _CW // _CW0
    n1 = (S // _TM1) * ncw
    n3 = S // _TM3
    dt = D // 128
    tpw = _CW // 128
    assert ncw == ppb == 4 and _CW <= D and _TM3 == 128 and 4 * Dh == 128

    def x_copy(i):
        rows = _ds(i * _XP, _XP, _XP)
        return pltpu.make_async_copy(
            x_hbm.at[0, rows, :], x_v.at[rows, :], sem_x.at[i])

    def wqkv_copy(c):
        cols = _ds(c * _CW, _CW, 128)
        return pltpu.make_async_copy(
            wqkv_hbm.at[:, cols], wqkv_v.at[:, cols], sem_w.at[c])

    def w0_copy(j):
        cols = _ds(j * _CW0, _CW0, 128)
        return pltpu.make_async_copy(
            wqkv_hbm.at[:, cols], wqkv_v.at[:, cols], sem_w.at[ncw + 5 + j])

    late_copies = [
        pltpu.make_async_copy(wo_hbm, wo_v, sem_w.at[ncw]),
        pltpu.make_async_copy(w1_hbm, w1_v, sem_w.at[ncw + 1]),
        pltpu.make_async_copy(w2_hbm, w2_v, sem_w.at[ncw + 2]),
        pltpu.make_async_copy(b1_hbm, b1_v, sem_w.at[ncw + 3]),
        pltpu.make_async_copy(b2_hbm, b2_v, sem_w.at[ncw + 4]),
    ]

    for i in range(ppb):
        x_copy(i).start()
    w0_copy(0).start()

    qscale = (Dh ** -0.5) * math.log2(math.e)

    def ln1(p):
        y = _layernorm(x_v[_ds(p * _XP, _XP, _XP), :].astype(f32))
        y1_s[_ds(p * (_XP // 2), _XP // 2, _XP // 2), :] = _pack(
            y.astype(bf16))

    def ln1_first(p, carry):
        x_copy(p).wait()
        ln1(p)
        return carry

    def transpose_tile(i, g):
        is_k = jnp.logical_and(g >= dt, g < 2 * dt)
        tt = jnp.where(is_k, 2 * dt, jnp.where(g < dt, g, g - dt))
        hrows = _ds(i * (_TM1 // 2), _TM1 // 2, _TM1 // 2)
        r = _unpack(nat_s[hrows, _ds(g * 128, 128, 128)])
        qvt_s[_ds(tt * 64, 64, 64), _ds(i * _TM1, _TM1, _TM1)] = _pack(r.T)

    def phase1_start(j, carry):
        w0_copy(j).wait()

        @pl.when(j == nsub0 - 1)
        def _():
            x_copy(ppb).wait()

        cols = _ds(j * _CW0, _CW0, 128)
        res = jnp.dot(_unpack(y1_s[0:_TM1 // 2, :]), wqkv_v[:, cols],
                      preferred_element_type=f32) * qscale
        nat_s[0:_TM1 // 2, cols] = _pack(res.astype(bf16))
        ln1(jnp.where(j == nsub0 - 1, ppb, ppb - 1))

        @pl.when(j == 0)
        def _():
            wqkv_copy(1).start()
            x_copy(ppb + 1).start()

        @pl.when(j == nsub0 - 1)
        def _():
            wqkv_copy(2).start()
            x_copy(ppb + 2).start()
        return carry

    def phase1(t, carry):
        i = t >> 2
        c = t & 3

        @pl.when(t < ncw)
        def _():
            wqkv_copy(t).wait()

        @pl.when(t + ppb < nxp)
        def _():
            x_copy(t + ppb).wait()

        for j in range(tpw):
            transpose_tile((t - 1) >> 2, ((t - 1) & 3) * tpw + j)
        hrows = _ds(i * (_TM1 // 2), _TM1 // 2, _TM1 // 2)
        res = jnp.dot(_unpack(y1_s[hrows, :]),
                      wqkv_v[:, _ds(c * _CW, _CW, 128)],
                      preferred_element_type=f32)
        for j in range(tpw):
            g = c * tpw + j
            r = res[:, j * 128:(j + 1) * 128] * jnp.where(g < dt, qscale, 1.0)
            nat_s[hrows, _ds(g * 128, 128, 128)] = _pack(r.astype(bf16))
        ln1(jnp.minimum(t + ppb, nxp - 1))

        @pl.when(t + 2 < ncw)
        def _():
            wqkv_copy(t + 2).start()

        @pl.when(t + ppb + 2 < nxp)
        def _():
            x_copy(t + ppb + 2).start()
        return carry

    lax.fori_loop(0, ppb, ln1_first, 0)
    for j in range(1, nsub0):
        w0_copy(j).start()
    x_copy(ppb).start()
    lax.fori_loop(0, nsub0, phase1_start, 0)
    lax.fori_loop(1, n1, phase1, 0)

    for c in late_copies:
        c.start()

    nkb = S // 128
    npc = S // _KP
    tpc = _QKC // 128
    ktp = _KP // 128
    hh = Dh // 2

    def stage_piece(n, nn, hq, hv, kc, qc, vc):
        rows = _ds(n * (S // 2 // nn), S // 2 // nn, S // 2 // nn)
        cols = _ds(n * (S // nn), S // nn, S // nn)
        kg = nat_s[rows, _ds(D + (hq >> 2) * 128, 128, 128)]
        kc[rows, :] = pltpu.roll(kg, (128 - (hq & 3) * Dh) & 127, 1)
        qc[:, cols] = qvt_s[_ds(hq * hh, hh, hh), cols]
        vc[:, cols] = qvt_s[_ds(D // 2 + hv * hh, hh, hh), cols]

    def make_qk(k_tile, q_cols, s_n, m_n):
        st = {}

        def qk(cb, kb):
            cols = _ds(cb * _QKC, _QKC, _QKC)
            if kb == 0:
                st['w'] = _unpack(jnp.concatenate(
                    [q_cols(cols), jnp.zeros((3 * hh, _QKC), jnp.uint32)],
                    axis=0))
            s = jnp.dot(_unpack(k_tile(kb)), st['w'],
                        preferred_element_type=f32)
            for t in range(tpc):
                s_n[cb * tpc + t, kb] = s[:, t * 128:(t + 1) * 128]
            mm = jnp.max(s.reshape(16, 8, _QKC), axis=0)
            st['m'] = mm if kb == 0 else jnp.maximum(st['m'], mm)
            if kb == nkb - 1:
                m_n[:, cols] = jnp.broadcast_to(
                    jnp.max(st['m'], axis=0, keepdims=True), (8, _QKC))
        return qk

    def make_sm(h, vc, s_c, m_c):
        st = {}

        def sm(ct, pc):
            cols = _ds(ct * 128, 128, 128)
            p = jnp.exp2(
                s_c[ct, pc * ktp:(pc + 1) * ktp].reshape(_KP // 8, 8, 128)
                - m_c[:, cols][None])
            for t in range(ktp):
                for r in reversed(range(8)):
                    pair = p[t * 16 + 2 * r] + p[t * 16 + 2 * r + 1]
                    first = pc == 0 and r == 7
                    st['l', t] = pair if first else st['l', t] + pair
            o = jnp.dot(_unpack(vc[:, pc * _KP:(pc + 1) * _KP]),
                        p.reshape(_KP, 128).astype(bf16),
                        preferred_element_type=f32)
            st['o'] = o if pc == 0 else o + st['o']
            if pc == npc - 1:
                l = st['l', 0]
                for t in range(1, ktp):
                    l = l + st['l', t]
                ot_s[_ds(h * Dh, Dh, Dh), cols] = (
                    st['o'] / jnp.sum(l, axis=0, keepdims=True))
        return sm

    def step(h, cur, nxt):
        (s_c, m_c, kc, qc, vc), (s_n, m_n, kn, qn, vn) = cur, nxt
        qk = make_qk(lambda kb: kc[kb * 64:(kb + 1) * 64, :],
                     lambda cols: qc[:, cols], s_n, m_n)
        sm = make_sm(h, vc, s_c, m_c)
        qk_ids = [(cb, kb) for cb in range(S // _QKC) for kb in range(nkb)]
        sm_ids = [(ct, pc) for ct in range(S // 128) for pc in range(npc)]
        assert len(qk_ids) == len(sm_ids)
        hq = jnp.minimum(h + 2, _H - 1)
        for n, (a, b) in enumerate(zip(qk_ids, sm_ids)):
            qk(*a)
            sm(*b)
            if n % 3 == 2 and n // 3 < 16:
                stage_piece(n // 3, 16, hq, h + 1, kn, qn, vn)

    buf_a = (s_a, m_a, kc_a, qc_a, vc_a)
    buf_b = (s_b, m_b, kc_b, qc_b, vc_b)

    def prologue(cb, carry):
        qk = make_qk(lambda kb: nat_s[kb * 64:(kb + 1) * 64, D:D + 128],
                     lambda cols: qvt_s[0:hh, cols], s_a, m_a)
        g0 = (ncw - 1) * tpw
        for kb in range(nkb):
            qk(cb, kb)
            if kb == 1:
                stage_piece(cb, S // _QKC, 1, 0, kc_a, qc_a, vc_a)
            if kb == 5:
                transpose_tile(S // _TM1 - 1, g0 + cb)
            if kb == 9:
                transpose_tile(S // _TM1 - 1,
                               g0 + jnp.minimum(cb + 4, tpw - 1))
        return carry

    def phase2(h, carry):
        @pl.when((h & 1) == 0)
        def _():
            step(h, buf_a, buf_b)

        @pl.when((h & 1) == 1)
        def _():
            step(h, buf_b, buf_a)
        return carry

    lax.fori_loop(0, S // _QKC, prologue, 0)
    lax.fori_loop(0, _H - 1, phase2, 0)

    for c in late_copies:
        c.wait()

    def out_copy(i):
        return pltpu.make_async_copy(
            out_v.at[i & 1], out_hbm.at[0, _ds(i * _TM3, _TM3, _TM3), :],
            sem_o.at[i & 1])

    def finish_a(h, slot):
        h_s[slot] = h
        y3_s[...] = _pack(_layernorm(_layernorm(h)).astype(bf16))

    def stage_a(i, slot):
        rows = _ds(i * _TM3, _TM3, _TM3)
        o = ot_s[:, rows].T.astype(bf16)
        finish_a(x_v[rows, :].astype(f32) + jnp.dot(
            o, wo_v[...], preferred_element_type=f32), slot)

    sm_last = make_sm(_H - 1, vc_b, s_b, m_b)
    k0 = D - 128
    o0 = ot_s[0:k0, 0:_TM3].T.astype(bf16)
    hs = []
    for n in range(dt):
        cs = slice(n * 128, (n + 1) * 128)
        hs.append(x_v[0:_TM3, cs].astype(f32) + jnp.dot(
            o0, wo_v[0:k0, cs], preferred_element_type=f32))
        sm_last(n // npc, n % npc)
    o1 = ot_s[k0:D, 0:_TM3].T.astype(bf16)
    finish_a(jnp.concatenate(hs, axis=1) + jnp.dot(
        o1, wo_v[k0:D, :], preferred_element_type=f32), 0)

    def mlp_block(i, last):
        sm31 = make_sm(_H - 1, vc_b, s_b, m_b)
        y = _unpack(y3_s[...])
        gs = []
        for c in range(F // _FC):
            a = jnp.dot(y, w1_v[:, c * _FC:(c + 1) * _FC],
                        preferred_element_type=f32)
            a = a + b1_v[pl.ds(c * _FC, _FC)].astype(f32).reshape(1, _FC)
            gs.append(jax.nn.gelu(a, approximate=True).astype(bf16))
            if not last and 1 <= c <= npc:
                sm31(jnp.minimum(i + 2, n3 - 1), c - 1)
        if not last:
            stage_a(i + 1, (i + 1) & 1)
        g = jnp.concatenate(gs, axis=1)
        r = jnp.dot(g, w2_v[...], preferred_element_type=f32)
        res = h_s[i & 1] + (r + b2_v[...].astype(f32).reshape(1, D))
        out_v[i & 1] = res.astype(bf16)
        out_copy(i).start()

    def phase3(i, carry):
        @pl.when(i >= 2)
        def _():
            out_copy(i - 2).wait()

        mlp_block(i, False)
        return carry

    lax.fori_loop(0, n3 - 1, phase3, 0)
    out_copy(n3 - 3).wait()
    mlp_block(n3 - 1, True)
    out_copy(n3 - 2).wait()
    out_copy(n3 - 1).wait()


@jax.jit
def pallas_sequential_preLN__softmax_full_mha__mixer_channel_mlp__prompt_kernel(
    A_x: jax.Array,
    A_wqkv: jax.Array,
    A_wo: jax.Array,
    B_x: jax.Array,
    B_w1: jax.Array,
    B_b1: jax.Array,
    B_w2: jax.Array,
    B_b2: jax.Array,
):
    del B_x
    B, S, D = A_x.shape
    F = B_w1.shape[1]
    assert B == 1
    f32, bf16, u32 = jnp.float32, jnp.bfloat16, jnp.uint32
    Dh = D // _H

    any_spec = pl.BlockSpec(memory_space=pl.ANY)
    s_shape = (S // 128, S // 128, 128, 128)
    scratch = [
        pltpu.VMEM((S, D), bf16),
        pltpu.VMEM((D, 3 * D + _WPAD), bf16),
        pltpu.VMEM((D, D), bf16),
        pltpu.VMEM((D, F), bf16),
        pltpu.VMEM((F,), bf16),
        pltpu.VMEM((F, D), bf16),
        pltpu.VMEM((D,), bf16),
        pltpu.VMEM((S // 2, D), u32),
        pltpu.VMEM((S // 2, 3 * D), u32),
        pltpu.VMEM((D + 64, S), u32),
        pltpu.VMEM((D, S), f32),
        pltpu.VMEM(s_shape, f32),
        pltpu.VMEM(s_shape, f32),
        pltpu.VMEM((8, S), f32),
        pltpu.VMEM((8, S), f32),
        pltpu.VMEM((S // 2, 128), u32),
        pltpu.VMEM((S // 2, 128), u32),
        pltpu.VMEM((Dh // 2, S), u32),
        pltpu.VMEM((Dh // 2, S), u32),
        pltpu.VMEM((Dh // 2, S), u32),
        pltpu.VMEM((Dh // 2, S), u32),
        pltpu.VMEM((2, _TM3, D), f32),
        pltpu.VMEM((_TM3 // 2, D), u32),
        pltpu.VMEM((2, _TM3, D), bf16),
        pltpu.SemaphoreType.DMA((S // _XP,)),
        pltpu.SemaphoreType.DMA((3 * D // _CW + 5 + _CW // _CW0,)),
        pltpu.SemaphoreType.DMA((2,)),
    ]
    return pl.pallas_call(
        functools.partial(_kernel, S=S, D=D, F=F),
        out_shape=jax.ShapeDtypeStruct((B, S, D), bf16),
        in_specs=[any_spec] * 7,
        out_specs=any_spec,
        scratch_shapes=scratch,
        compiler_params=pltpu.CompilerParams(
            vmem_limit_bytes=120 * 1024 * 1024,
            disable_bounds_checks=True,
            disable_semaphore_checks=True),
    )(A_x, A_wqkv, A_wo, B_w1, B_b1, B_w2, B_b2)
```

```python
import functools
import math

import jax
import jax.numpy as jnp
from jax import lax
import jax.experimental.pallas as pl
import jax.experimental.pallas.tpu as pltpu

_EPS = 1e-5
_H = 32
_TM1 = 512
_CW = 768
_CW0 = 256
_XP = 128
_TM3 = 128
_FC = 512
_QKC = 512
_KP = 512
_STAG = 16
_LAG = 2
_WPAD = 128


def _layernorm(x):
    m = jnp.mean(x, axis=-1, keepdims=True)
    xc = x - m
    v = jnp.mean(xc * xc, axis=-1, keepdims=True)
    return xc * lax.rsqrt(v + _EPS)


def _pack(x):
    return pltpu.bitcast(x, jnp.uint32)


def _unpack(x):
    return pltpu.bitcast(x, jnp.bfloat16)


def _ds(start, size, align):
    if not isinstance(start, int):
        start = pl.multiple_of(start, align)
    return pl.ds(start, size)


def _kernel(x_hbm, wqkv_hbm, wo_hbm, w1_hbm, b1_hbm, w2_hbm, b2_hbm, out_hbm,
            x_v, wqkv_v, wo_v, w1_v, b1_v, w2_v, b2_v,
            y1_s, nat_s, qvt_s, ot_s, s_a, s_b, m_a, m_b,
            kc_a, kc_b, qc_a, qc_b, vc_a, vc_b, zero_s, h_s, y3_s, out_v,
            sem_x, sem_w, sem_o, *, S, D, F):
    f32, bf16 = jnp.float32, jnp.bfloat16
    Dh = D // _H
    nxp = S // _XP
    ppb = _TM1 // _XP
    ncw = 3 * D // _CW
    nsub0 = _CW // _CW0
    n1 = (S // _TM1) * ncw
    n3 = S // _TM3
    dt = D // 128
    tpw = _CW // 128
    assert ncw == ppb == 4 and _CW <= D and _TM3 == 128 and 4 * Dh == 128

    def x_copy(i):
        rows = _ds(i * _XP, _XP, _XP)
        return pltpu.make_async_copy(
            x_hbm.at[0, rows, :], x_v.at[rows, :], sem_x.at[i])

    def wqkv_copy(c):
        cols = _ds(c * _CW, _CW, 128)
        return pltpu.make_async_copy(
            wqkv_hbm.at[:, cols], wqkv_v.at[:, cols], sem_w.at[c])

    def w0_copy(j):
        cols = _ds(j * _CW0, _CW0, 128)
        return pltpu.make_async_copy(
            wqkv_hbm.at[:, cols], wqkv_v.at[:, cols], sem_w.at[ncw + 5 + j])

    late_copies = [
        pltpu.make_async_copy(wo_hbm, wo_v, sem_w.at[ncw]),
        pltpu.make_async_copy(w1_hbm, w1_v, sem_w.at[ncw + 1]),
        pltpu.make_async_copy(w2_hbm, w2_v, sem_w.at[ncw + 2]),
        pltpu.make_async_copy(b1_hbm, b1_v, sem_w.at[ncw + 3]),
        pltpu.make_async_copy(b2_hbm, b2_v, sem_w.at[ncw + 4]),
    ]

    for i in range(ppb):
        x_copy(i).start()
    w0_copy(0).start()
    zero_s[...] = jnp.zeros((8, 128), jnp.uint32)

    qscale = (Dh ** -0.5) * math.log2(math.e)

    def ln1(p):
        y = _layernorm(x_v[_ds(p * _XP, _XP, _XP), :].astype(f32))
        y1_s[_ds(p * (_XP // 2), _XP // 2, _XP // 2), :] = _pack(
            y.astype(bf16))

    def ln1_first(p, carry):
        x_copy(p).wait()
        ln1(p)
        return carry

    def transpose_tile(i, g):
        is_k = jnp.logical_and(g >= dt, g < 2 * dt)
        tt = jnp.where(is_k, 2 * dt, jnp.where(g < dt, g, g - dt))
        hrows = _ds(i * (_TM1 // 2), _TM1 // 2, _TM1 // 2)
        r = _unpack(nat_s[hrows, _ds(g * 128, 128, 128)])
        qvt_s[_ds(tt * 64, 64, 64), _ds(i * _TM1, _TM1, _TM1)] = _pack(r.T)

    def phase1_start(j, carry):
        w0_copy(j).wait()

        @pl.when(j == nsub0 - 1)
        def _():
            x_copy(ppb).wait()

        cols = _ds(j * _CW0, _CW0, 128)
        res = jnp.dot(_unpack(y1_s[0:_TM1 // 2, :]), wqkv_v[:, cols],
                      preferred_element_type=f32) * qscale
        nat_s[0:_TM1 // 2, cols] = _pack(res.astype(bf16))
        ln1(jnp.where(j == nsub0 - 1, ppb, ppb - 1))

        @pl.when(j == 0)
        def _():
            wqkv_copy(1).start()
            x_copy(ppb + 1).start()

        @pl.when(j == nsub0 - 1)
        def _():
            wqkv_copy(2).start()
            x_copy(ppb + 2).start()
        return carry

    def phase1(t, carry):
        i = t >> 2
        c = t & 3

        @pl.when(t < ncw)
        def _():
            wqkv_copy(t).wait()

        @pl.when(t + ppb < nxp)
        def _():
            x_copy(t + ppb).wait()

        for j in range(tpw):
            transpose_tile((t - 1) >> 2, ((t - 1) & 3) * tpw + j)
        hrows = _ds(i * (_TM1 // 2), _TM1 // 2, _TM1 // 2)
        res = jnp.dot(_unpack(y1_s[hrows, :]),
                      wqkv_v[:, _ds(c * _CW, _CW, 128)],
                      preferred_element_type=f32)
        for j in range(tpw):
            g = c * tpw + j
            r = res[:, j * 128:(j + 1) * 128] * jnp.where(g < dt, qscale, 1.0)
            nat_s[hrows, _ds(g * 128, 128, 128)] = _pack(r.astype(bf16))
        ln1(jnp.minimum(t + ppb, nxp - 1))

        @pl.when(t + 2 < ncw)
        def _():
            wqkv_copy(t + 2).start()

        @pl.when(t + ppb + 2 < nxp)
        def _():
            x_copy(t + ppb + 2).start()
        return carry

    lax.fori_loop(0, ppb, ln1_first, 0)
    for j in range(1, nsub0):
        w0_copy(j).start()
    x_copy(ppb).start()
    lax.fori_loop(0, nsub0, phase1_start, 0)
    lax.fori_loop(1, n1, phase1, 0)

    for c in late_copies:
        c.start()

    nkb = S // 128
    npc = S // _KP
    tpc = _QKC // 128
    ktp = _KP // 128
    hh = Dh // 2

    def stage_piece(n, nn, hq, hv, kc, qc, vc):
        rows = _ds(n * (S // 2 // nn), S // 2 // nn, S // 2 // nn)
        cols = _ds(n * (S // nn), S // nn, S // nn)
        kg = nat_s[rows, _ds(D + (hq >> 2) * 128, 128, 128)]
        kc[rows, :] = pltpu.roll(kg, (128 - (hq & 3) * Dh) & 127, 1)
        z = jnp.tile(zero_s[...], (hh // 8, S // nn // 128))
        qc[:, cols] = qvt_s[_ds(hq * hh, hh, hh), cols] | z
        vc[:, cols] = qvt_s[_ds(D // 2 + hv * hh, hh, hh), cols] | z

    def make_qk(k_tile, q_cols, s_n, m_n, hist=None):
        st = {}

        def qk(cb, kb):
            cols = _ds(cb * _QKC, _QKC, _QKC)
            if kb == 0:
                st['w'] = _unpack(jnp.concatenate(
                    [q_cols(cols), jnp.zeros((3 * hh, _QKC), jnp.uint32)],
                    axis=0))
            s = jnp.dot(_unpack(k_tile(kb)), st['w'],
                        preferred_element_type=f32)
            if hist is not None:
                hist.append(s[:, 0:128])
            for t in range(tpc):
                s_n[cb * tpc + t, kb] = s[:, t * 128:(t + 1) * 128]
            mm = jnp.max(s.reshape(16, 8, _QKC), axis=0)
            st['m'] = mm if kb == 0 else jnp.maximum(st['m'], mm)
            if kb == nkb - 1:
                m_n[:, cols] = jnp.broadcast_to(
                    jnp.max(st['m'], axis=0, keepdims=True), (8, _QKC))
        return qk

    def make_sm(h, v_cols, s_c, m_c, hist=None, pace=False):
        st = {}

        def sm(ct, pc):
            cols = _ds(ct * 128, 128, 128)
            mv = m_c[:, cols]
            if pace:
                src = hist[-_LAG]
                mvs = jnp.stack([
                    mv + jnp.minimum(jnp.abs(
                        src[(7 - r) * _STAG:(7 - r) * _STAG + 8]), 0.0)
                    for r in range(8)], axis=0)
                p = jnp.exp2(
                    s_c[ct, pc * ktp:(pc + 1) * ktp].reshape(ktp, 8, 2, 8, 128)
                    - mvs[None, :, None]).reshape(_KP // 8, 8, 128)
            else:
                p = jnp.exp2(
                    s_c[ct, pc * ktp:(pc + 1) * ktp].reshape(_KP // 8, 8, 128)
                    - mv[None])
            for t in range(ktp):
                for r in reversed(range(8)):
                    pair = p[t * 16 + 2 * r] + p[t * 16 + 2 * r + 1]
                    first = pc == 0 and r == 7
                    st['l', t] = pair if first else st['l', t] + pair
            o = jnp.dot(_unpack(v_cols(slice(pc * _KP, (pc + 1) * _KP))),
                        p.reshape(_KP, 128).astype(bf16),
                        preferred_element_type=f32)
            st['o'] = o if pc == 0 else o + st['o']
            if pc == npc - 1:
                l = st['l', 0]
                for t in range(1, ktp):
                    l = l + st['l', t]
                ot_s[_ds(h * Dh, Dh, Dh), cols] = (
                    st['o'] / jnp.sum(l, axis=0, keepdims=True))
        return sm

    def step(h, cur, nxt, hist, pace):
        (s_c, m_c, kc, qc, vc), (s_n, m_n, kn, qn, vn) = cur, nxt
        qk = make_qk(lambda kb: kc[kb * 64:(kb + 1) * 64, :],
                     lambda cols: qc[:, cols], s_n, m_n, hist)
        sm = make_sm(h, lambda cols: vc[:, cols], s_c, m_c, hist, pace)
        qk_ids = [(cb, kb) for cb in range(S // _QKC) for kb in range(nkb)]
        sm_ids = [(ct, pc) for ct in range(S // 128) for pc in range(npc)]
        assert len(qk_ids) == len(sm_ids)
        hq = jnp.minimum(h + 2, _H - 1)
        for n, (a, b) in enumerate(zip(qk_ids, sm_ids)):
            qk(*a)
            sm(*b)
            if n % 3 == 2 and n // 3 < 16:
                stage_piece(n // 3, 16, hq, h + 1, kn, qn, vn)

    buf_a = (s_a, m_a, kc_a, qc_a, vc_a)
    buf_b = (s_b, m_b, kc_b, qc_b, vc_b)

    def first_heads(cb, carry):
        def k_tile(kb):
            return nat_s[kb * 64:(kb + 1) * 64, D:D + 128]

        hist = []
        qk0 = make_qk(k_tile, lambda cols: qvt_s[0:hh, cols], s_a, m_a, hist)
        qk1 = make_qk(lambda kb: pltpu.roll(k_tile(kb), 128 - Dh, 1),
                      lambda cols: qvt_s[hh:2 * hh, cols], s_b, m_b, hist)
        sm0 = make_sm(0, lambda cols: qvt_s[D // 2:D // 2 + hh, cols],
                      s_a, m_a, hist, True)
        g0 = (ncw - 1) * tpw
        for kb in range(nkb):
            qk0(cb, kb)
            if kb == 1:
                stage_piece(cb, S // _QKC, 2, 1, kc_b, qc_b, vc_b)
            if kb == 5:
                transpose_tile(S // _TM1 - 1, g0 + cb)
            if kb == 9:
                transpose_tile(S // _TM1 - 1,
                               g0 + jnp.minimum(cb + 4, tpw - 1))
        qk1(cb, 0)
        for kb in range(1, nkb):
            qk1(cb, kb)
            sm0(cb * tpc + (kb - 1) // npc, (kb - 1) % npc)
        sm0(cb * tpc + tpc - 1, npc - 1)
        return carry

    def phase2(i, carry):
        hist = []
        step(2 * i + 1, buf_b, buf_a, hist, False)
        step(2 * i + 2, buf_a, buf_b, hist, True)
        return carry

    lax.fori_loop(0, S // _QKC, first_heads, 0)
    lax.fori_loop(0, (_H - 2) // 2, phase2, 0)

    for c in late_copies:
        c.wait()

    def out_copy(i):
        return pltpu.make_async_copy(
            out_v.at[i & 1], out_hbm.at[0, _ds(i * _TM3, _TM3, _TM3), :],
            sem_o.at[i & 1])

    def finish_a(h, slot):
        h_s[slot] = h
        y3_s[...] = _pack(_layernorm(_layernorm(h)).astype(bf16))

    def stage_a(i, slot):
        rows = _ds(i * _TM3, _TM3, _TM3)
        o = ot_s[:, rows].T.astype(bf16)
        finish_a(x_v[rows, :].astype(f32) + jnp.dot(
            o, wo_v[...], preferred_element_type=f32), slot)

    sm_last = make_sm(_H - 1, lambda cols: vc_b[:, cols], s_b, m_b)
    k0 = D - 128
    o0 = ot_s[0:k0, 0:_TM3].T.astype(bf16)
    hs = []
    for n in range(dt):
        cs = slice(n * 128, (n + 1) * 128)
        hs.append(x_v[0:_TM3, cs].astype(f32) + jnp.dot(
            o0, wo_v[0:k0, cs], preferred_element_type=f32))
        sm_last(n // npc, n % npc)
    o1 = ot_s[k0:D, 0:_TM3].T.astype(bf16)
    finish_a(jnp.concatenate(hs, axis=1) + jnp.dot(
        o1, wo_v[k0:D, :], preferred_element_type=f32), 0)

    def mlp_block(i, last):
        sm31 = make_sm(_H - 1, lambda cols: vc_b[:, cols], s_b, m_b)
        y = _unpack(y3_s[...])
        gs = []
        for c in range(F // _FC):
            a = jnp.dot(y, w1_v[:, c * _FC:(c + 1) * _FC],
                        preferred_element_type=f32)
            a = a + b1_v[pl.ds(c * _FC, _FC)].astype(f32).reshape(1, _FC)
            gs.append(jax.nn.gelu(a, approximate=True).astype(bf16))
            if not last and 1 <= c <= npc:
                sm31(jnp.minimum(i + 2, n3 - 1), c - 1)
        if not last:
            stage_a(i + 1, (i + 1) & 1)
        g = jnp.concatenate(gs, axis=1)
        r = jnp.dot(g, w2_v[...], preferred_element_type=f32)
        res = h_s[i & 1] + (r + b2_v[...].astype(f32).reshape(1, D))
        out_v[i & 1] = res.astype(bf16)
        out_copy(i).start()

    def phase3(i, carry):
        @pl.when(i >= 2)
        def _():
            out_copy(i - 2).wait()

        mlp_block(i, False)
        return carry

    lax.fori_loop(0, n3 - 1, phase3, 0)
    out_copy(n3 - 3).wait()
    mlp_block(n3 - 1, True)
    out_copy(n3 - 2).wait()
    out_copy(n3 - 1).wait()


@jax.jit
def pallas_sequential_preLN__softmax_full_mha__mixer_channel_mlp__prompt_kernel(
    A_x: jax.Array,
    A_wqkv: jax.Array,
    A_wo: jax.Array,
    B_x: jax.Array,
    B_w1: jax.Array,
    B_b1: jax.Array,
    B_w2: jax.Array,
    B_b2: jax.Array,
):
    del B_x
    B, S, D = A_x.shape
    F = B_w1.shape[1]
    assert B == 1
    f32, bf16, u32 = jnp.float32, jnp.bfloat16, jnp.uint32
    Dh = D // _H

    any_spec = pl.BlockSpec(memory_space=pl.ANY)
    s_shape = (S // 128, S // 128, 128, 128)
    scratch = [
        pltpu.VMEM((S, D), bf16),
        pltpu.VMEM((D, 3 * D + _WPAD), bf16),
        pltpu.VMEM((D, D), bf16),
        pltpu.VMEM((D, F), bf16),
        pltpu.VMEM((F,), bf16),
        pltpu.VMEM((F, D), bf16),
        pltpu.VMEM((D,), bf16),
        pltpu.VMEM((S // 2, D), u32),
        pltpu.VMEM((S // 2, 3 * D), u32),
        pltpu.VMEM((D + 64, S), u32),
        pltpu.VMEM((D, S), f32),
        pltpu.VMEM(s_shape, f32),
        pltpu.VMEM(s_shape, f32),
        pltpu.VMEM((8, S), f32),
        pltpu.VMEM((8, S), f32),
        pltpu.VMEM((S // 2, 128), u32),
        pltpu.VMEM((S // 2, 128), u32),
        pltpu.VMEM((Dh // 2, S), u32),
        pltpu.VMEM((Dh // 2, S), u32),
        pltpu.VMEM((Dh // 2, S), u32),
        pltpu.VMEM((Dh // 2, S), u32),
        pltpu.VMEM((8, 128), u32),
        pltpu.VMEM((2, _TM3, D), f32),
        pltpu.VMEM((_TM3 // 2, D), u32),
        pltpu.VMEM((2, _TM3, D), bf16),
        pltpu.SemaphoreType.DMA((S // _XP,)),
        pltpu.SemaphoreType.DMA((3 * D // _CW + 5 + _CW // _CW0,)),
        pltpu.SemaphoreType.DMA((2,)),
    ]
    return pl.pallas_call(
        functools.partial(_kernel, S=S, D=D, F=F),
        out_shape=jax.ShapeDtypeStruct((B, S, D), bf16),
        in_specs=[any_spec] * 7,
        out_specs=any_spec,
        scratch_shapes=scratch,
        compiler_params=pltpu.CompilerParams(
            vmem_limit_bytes=120 * 1024 * 1024,
            disable_bounds_checks=True,
            disable_semaphore_checks=True),
    )(A_x, A_wqkv, A_wo, B_w1, B_b1, B_w2, B_b2)
```

```python
import functools
import math

import jax
import jax.numpy as jnp
from jax import lax
import jax.experimental.pallas as pl
import jax.experimental.pallas.tpu as pltpu

_EPS = 1e-5
_H = 32
_TM1 = 512
_CW = 768
_CW0 = 256
_XP = 128
_TM3 = 128
_FC = 512
_QKC = 512
_KP = 512
_VT = (3, 7, 11, 15)
_WPAD = 128


def _layernorm(x):
    m = jnp.mean(x, axis=-1, keepdims=True)
    xc = x - m
    v = jnp.mean(xc * xc, axis=-1, keepdims=True)
    return xc * lax.rsqrt(v + _EPS)


def _pack(x):
    return pltpu.bitcast(x, jnp.uint32)


def _unpack(x):
    return pltpu.bitcast(x, jnp.bfloat16)


def _zero_after(x):
    return jnp.minimum(jnp.abs(x), 0.0)


def _ds(start, size, align):
    if not isinstance(start, int):
        start = pl.multiple_of(start, align)
    return pl.ds(start, size)


def _kernel(x_hbm, wqkv_hbm, wo_hbm, w1_hbm, b1_hbm, w2_hbm, b2_hbm, out_hbm,
            x_v, wqkv_v, wo_v, w1_v, b1_v, w2_v, b2_v,
            y1_s, nat_s, qvt_s, ot_s, s_a, s_b, m_a, m_b,
            kc_a, kc_b, qc_a, qc_b, vc_a, vc_b, qf_a, qf_b, zero_s, h_s, y3_s, out_v,
            sem_x, sem_w, sem_o, *, S, D, F):
    f32, bf16 = jnp.float32, jnp.bfloat16
    Dh = D // _H
    nxp = S // _XP
    ppb = _TM1 // _XP
    ncw = 3 * D // _CW
    nsub0 = _CW // _CW0
    n1 = (S // _TM1) * ncw
    n3 = S // _TM3
    dt = D // 128
    tpw = _CW // 128
    assert ncw == ppb == 4 and _CW <= D and _TM3 == 128 and 4 * Dh == 128

    def x_copy(i):
        rows = _ds(i * _XP, _XP, _XP)
        return pltpu.make_async_copy(
            x_hbm.at[0, rows, :], x_v.at[rows, :], sem_x.at[i])

    def wqkv_copy(c):
        cols = _ds(c * _CW, _CW, 128)
        return pltpu.make_async_copy(
            wqkv_hbm.at[:, cols], wqkv_v.at[:, cols], sem_w.at[c])

    def w0_copy(j):
        cols = _ds(j * _CW0, _CW0, 128)
        return pltpu.make_async_copy(
            wqkv_hbm.at[:, cols], wqkv_v.at[:, cols], sem_w.at[ncw + 5 + j])

    late_copies = [
        pltpu.make_async_copy(wo_hbm, wo_v, sem_w.at[ncw]),
        pltpu.make_async_copy(w1_hbm, w1_v, sem_w.at[ncw + 1]),
        pltpu.make_async_copy(w2_hbm, w2_v, sem_w.at[ncw + 2]),
        pltpu.make_async_copy(b1_hbm, b1_v, sem_w.at[ncw + 3]),
        pltpu.make_async_copy(b2_hbm, b2_v, sem_w.at[ncw + 4]),
    ]

    for i in range(ppb):
        x_copy(i).start()
    w0_copy(0).start()
    zero_s[...] = jnp.zeros((8, 128), jnp.uint32)

    qscale = (Dh ** -0.5) * math.log2(math.e)

    def ln1(p):
        y = _layernorm(x_v[_ds(p * _XP, _XP, _XP), :].astype(f32))
        y1_s[_ds(p * (_XP // 2), _XP // 2, _XP // 2), :] = _pack(
            y.astype(bf16))

    def ln1_first(p, carry):
        x_copy(p).wait()
        ln1(p)
        return carry

    def transpose_tile(i, g):
        is_k = jnp.logical_and(g >= dt, g < 2 * dt)
        tt = jnp.where(is_k, 2 * dt, jnp.where(g < dt, g, g - dt))
        hrows = _ds(i * (_TM1 // 2), _TM1 // 2, _TM1 // 2)
        r = _unpack(nat_s[hrows, _ds(g * 128, 128, 128)])
        qvt_s[_ds(tt * 64, 64, 64), _ds(i * _TM1, _TM1, _TM1)] = _pack(r.T)

    def phase1_start(j, carry):
        w0_copy(j).wait()

        @pl.when(j == nsub0 - 1)
        def _():
            x_copy(ppb).wait()

        cols = _ds(j * _CW0, _CW0, 128)
        res = jnp.dot(_unpack(y1_s[0:_TM1 // 2, :]), wqkv_v[:, cols],
                      preferred_element_type=f32) * qscale
        nat_s[0:_TM1 // 2, cols] = _pack(res.astype(bf16))
        ln1(jnp.where(j == nsub0 - 1, ppb, ppb - 1))

        @pl.when(j == 0)
        def _():
            wqkv_copy(1).start()
            x_copy(ppb + 1).start()

        @pl.when(j == nsub0 - 1)
        def _():
            wqkv_copy(2).start()
            x_copy(ppb + 2).start()
        return carry

    def phase1(t, carry):
        i = t >> 2
        c = t & 3

        @pl.when(t < ncw)
        def _():
            wqkv_copy(t).wait()

        @pl.when(t + ppb < nxp)
        def _():
            x_copy(t + ppb).wait()

        for j in range(tpw):
            transpose_tile((t - 1) >> 2, ((t - 1) & 3) * tpw + j)
        hrows = _ds(i * (_TM1 // 2), _TM1 // 2, _TM1 // 2)
        res = jnp.dot(_unpack(y1_s[hrows, :]),
                      wqkv_v[:, _ds(c * _CW, _CW, 128)],
                      preferred_element_type=f32)
        for j in range(tpw):
            g = c * tpw + j
            r = res[:, j * 128:(j + 1) * 128] * jnp.where(g < dt, qscale, 1.0)
            nat_s[hrows, _ds(g * 128, 128, 128)] = _pack(r.astype(bf16))
        ln1(jnp.minimum(t + ppb, nxp - 1))

        @pl.when(t + 2 < ncw)
        def _():
            wqkv_copy(t + 2).start()

        @pl.when(t + ppb + 2 < nxp)
        def _():
            x_copy(t + ppb + 2).start()
        return carry

    lax.fori_loop(0, ppb, ln1_first, 0)
    for j in range(1, nsub0):
        w0_copy(j).start()
    x_copy(ppb).start()
    lax.fori_loop(0, nsub0, phase1_start, 0)
    lax.fori_loop(1, n1, phase1, 0)

    for c in late_copies:
        c.start()

    nkb = S // 128
    npc = S // _KP
    tpc = _QKC // 128
    ktp = _KP // 128
    hh = Dh // 2

    def stage_piece(n, nn, hq, hv, kc, qc, vc, qf):
        rows = _ds(n * (S // 2 // nn), S // 2 // nn, S // 2 // nn)
        cols = _ds(n * (S // nn), S // nn, S // nn)
        kg = nat_s[rows, _ds(D + (hq >> 2) * 128, 128, 128)]
        kc[rows, :] = pltpu.roll(kg, (128 - (hq & 3) * Dh) & 127, 1)
        z = jnp.tile(zero_s[...], (hh // 8, S // nn // 128))
        qh = qvt_s[_ds(hq * hh, hh, hh), cols] | z
        qc[:, cols] = qh
        qf[:, cols] = _unpack(qh).astype(f32)
        vc[:, cols] = qvt_s[_ds(D // 2 + hv * hh, hh, hh), cols] | z

    def make_qk(k_tile, q_cols, s_n, m_n, hist, qf=None):
        st = {}

        def qk(cb, kb):
            cols = _ds(cb * _QKC, _QKC, _QKC)
            if kb == 0:
                st['w'] = _unpack(jnp.concatenate(
                    [q_cols(cols), jnp.zeros((3 * hh, _QKC), jnp.uint32)],
                    axis=0))
            nr = 112 if (qf is not None and kb in _VT) else 128
            s = jnp.dot(_unpack(k_tile(kb)[0:nr // 2]), st['w'],
                        preferred_element_type=f32)
            prev = hist[-1] if hist else None
            hist.append(s[:, 0:128])
            for t in range(tpc):
                s_n[cb * tpc + t, kb, 0:nr] = s[:, t * 128:(t + 1) * 128]
            mm = jnp.max(s.reshape(nr // 8, 8, _QKC), axis=0)
            st['m'] = mm if kb == 0 else jnp.maximum(st['m'], mm)
            if qf is not None:
                per = len(_VT) * 2 * Dh // nkb
                for e in range(kb * per, (kb + 1) * per):
                    kt, g, d = _VT[e // (2 * Dh)], (e // Dh) % 2, e % Dh
                    el = e - kb * per
                    if d == 0:
                        st['kf'] = _unpack(k_tile(kt)[56:64]).astype(f32)[
                            g * 8:(g + 1) * 8]
                    if el % 2 == 0:
                        st['kp'] = st['kf']
                        if prev is not None:
                            j = (el * 96 // per) // 8 * 8
                            st['kp'] = st['kf'] + _zero_after(prev[j:j + 8])
                    kcol = jnp.broadcast_to(st['kp'][:, d:d + 1], (8, 128))
                    for t in range(tpc):
                        c0 = cb * _QKC + t * 128
                        pr = kcol * qf[d:d + 1, c0:c0 + 128]
                        st['acc', t] = pr if d == 0 else st['acc', t] + pr
                    if d == Dh - 1:
                        r0 = 112 + g * 8
                        for t in range(tpc):
                            s_n[cb * tpc + t, kt, r0:r0 + 8] = st['acc', t]
                        st['m'] = jnp.maximum(st['m'], jnp.concatenate(
                            [st['acc', t] for t in range(tpc)], axis=1))
            if kb == nkb - 1:
                m_n[:, cols] = jnp.broadcast_to(
                    jnp.max(st['m'], axis=0, keepdims=True), (8, _QKC))
        return qk

    def make_sm(h, v_cols, s_c, m_c, hist=None, pace=False):
        st = {}

        def sm(ct, pc):
            cols = _ds(ct * 128, 128, 128)
            mv = m_c[:, cols]
            if pace:
                src = hist[-2]
                mvs = jnp.stack([
                    mv + _zero_after(src[(7 - r) * 14:(7 - r) * 14 + 8])
                    for r in range(8)], axis=0)
                p = jnp.exp2(
                    s_c[ct, pc * ktp:(pc + 1) * ktp].reshape(ktp, 8, 2, 8, 128)
                    - mvs[None, :, None]).reshape(_KP // 8, 8, 128)
            else:
                p = jnp.exp2(
                    s_c[ct, pc * ktp:(pc + 1) * ktp].reshape(_KP // 8, 8, 128)
                    - mv[None])
            for t in range(ktp):
                for r in reversed(range(8)):
                    pair = p[t * 16 + 2 * r] + p[t * 16 + 2 * r + 1]
                    first = pc == 0 and r == 7
                    st['l', t] = pair if first else st['l', t] + pair
            o = jnp.dot(_unpack(v_cols(slice(pc * _KP, (pc + 1) * _KP))),
                        p.reshape(_KP, 128).astype(bf16),
                        preferred_element_type=f32)
            st['o'] = o if pc == 0 else o + st['o']
            if pc == npc - 1:
                l = st['l', 0]
                for t in range(1, ktp):
                    l = l + st['l', t]
                ot_s[_ds(h * Dh, Dh, Dh), cols] = (
                    st['o'] / jnp.sum(l, axis=0, keepdims=True))
        return sm

    def step(h, cur, nxt, hist, pace):
        (s_c, m_c, kc, qc, vc, qf), (s_n, m_n, kn, qn, vn, qfn) = cur, nxt
        qk = make_qk(lambda kb: kc[kb * 64:(kb + 1) * 64, :],
                     lambda cols: qc[:, cols], s_n, m_n, hist, qf)
        sm = make_sm(h, lambda cols: vc[:, cols], s_c, m_c, hist, pace)
        qk_ids = [(cb, kb) for cb in range(S // _QKC) for kb in range(nkb)]
        sm_ids = [(ct, pc) for ct in range(S // 128) for pc in range(npc)]
        assert len(qk_ids) == len(sm_ids)
        hq = jnp.minimum(h + 2, _H - 1)
        for n, (a, b) in enumerate(zip(qk_ids, sm_ids)):
            qk(*a)
            sm(*b)
            if n % 3 == 2 and n // 3 < 16:
                stage_piece(n // 3, 16, hq, h + 1, kn, qn, vn, qfn)

    buf_a = (s_a, m_a, kc_a, qc_a, vc_a, qf_a)
    buf_b = (s_b, m_b, kc_b, qc_b, vc_b, qf_b)

    def first_heads(cb, carry):
        def k_tile(kb):
            return nat_s[kb * 64:(kb + 1) * 64, D:D + 128]

        hist = []
        qk0 = make_qk(k_tile, lambda cols: qvt_s[0:hh, cols], s_a, m_a, hist)
        qk1 = make_qk(lambda kb: pltpu.roll(k_tile(kb), 128 - Dh, 1),
                      lambda cols: qvt_s[hh:2 * hh, cols], s_b, m_b, hist)
        sm0 = make_sm(0, lambda cols: qvt_s[D // 2:D // 2 + hh, cols],
                      s_a, m_a, hist, True)
        g0 = (ncw - 1) * tpw
        for kb in range(nkb):
            qk0(cb, kb)
            if kb == 1:
                stage_piece(cb, S // _QKC, 2, 1, kc_b, qc_b, vc_b, qf_b)
            if kb == 5:
                transpose_tile(S // _TM1 - 1, g0 + cb)
            if kb == 9:
                transpose_tile(S // _TM1 - 1,
                               g0 + jnp.minimum(cb + 4, tpw - 1))
        qk1(cb, 0)
        for kb in range(1, nkb):
            qk1(cb, kb)
            sm0(cb * tpc + (kb - 1) // npc, (kb - 1) % npc)
        sm0(cb * tpc + tpc - 1, npc - 1)
        return carry

    def phase2(i, carry):
        hist = []
        step(2 * i + 1, buf_b, buf_a, hist, False)
        step(2 * i + 2, buf_a, buf_b, hist, True)
        return carry

    lax.fori_loop(0, S // _QKC, first_heads, 0)
    lax.fori_loop(0, (_H - 2) // 2, phase2, 0)

    for c in late_copies:
        c.wait()

    def out_copy(i):
        return pltpu.make_async_copy(
            out_v.at[i & 1], out_hbm.at[0, _ds(i * _TM3, _TM3, _TM3), :],
            sem_o.at[i & 1])

    def finish_a(h, slot):
        h_s[slot] = h
        y3_s[...] = _pack(_layernorm(_layernorm(h)).astype(bf16))

    def stage_a(i, slot):
        rows = _ds(i * _TM3, _TM3, _TM3)
        o = ot_s[:, rows].T.astype(bf16)
        finish_a(x_v[rows, :].astype(f32) + jnp.dot(
            o, wo_v[...], preferred_element_type=f32), slot)

    sm_last = make_sm(_H - 1, lambda cols: vc_b[:, cols], s_b, m_b)
    k0 = D - 128
    o0 = ot_s[0:k0, 0:_TM3].T.astype(bf16)
    hs = []
    for n in range(dt):
        cs = slice(n * 128, (n + 1) * 128)
        hs.append(x_v[0:_TM3, cs].astype(f32) + jnp.dot(
            o0, wo_v[0:k0, cs], preferred_element_type=f32))
        sm_last(n // npc, n % npc)
    o1 = ot_s[k0:D, 0:_TM3].T.astype(bf16)
    finish_a(jnp.concatenate(hs, axis=1) + jnp.dot(
        o1, wo_v[k0:D, :], preferred_element_type=f32), 0)

    def mlp_block(i, last):
        sm31 = make_sm(_H - 1, lambda cols: vc_b[:, cols], s_b, m_b)
        y = _unpack(y3_s[...])
        gs = []
        for c in range(F // _FC):
            a = jnp.dot(y, w1_v[:, c * _FC:(c + 1) * _FC],
                        preferred_element_type=f32)
            a = a + b1_v[pl.ds(c * _FC, _FC)].astype(f32).reshape(1, _FC)
            gs.append(jax.nn.gelu(a, approximate=True).astype(bf16))
            if not last and 1 <= c <= npc:
                sm31(jnp.minimum(i + 2, n3 - 1), c - 1)
        if not last:
            stage_a(i + 1, (i + 1) & 1)
        g = jnp.concatenate(gs, axis=1)
        r = jnp.dot(g, w2_v[...], preferred_element_type=f32)
        res = h_s[i & 1] + (r + b2_v[...].astype(f32).reshape(1, D))
        out_v[i & 1] = res.astype(bf16)
        out_copy(i).start()

    def phase3(i, carry):
        @pl.when(i >= 2)
        def _():
            out_copy(i - 2).wait()

        mlp_block(i, False)
        return carry

    lax.fori_loop(0, n3 - 1, phase3, 0)
    out_copy(n3 - 3).wait()
    mlp_block(n3 - 1, True)
    out_copy(n3 - 2).wait()
    out_copy(n3 - 1).wait()


@jax.jit
def pallas_sequential_preLN__softmax_full_mha__mixer_channel_mlp__prompt_kernel(
    A_x: jax.Array,
    A_wqkv: jax.Array,
    A_wo: jax.Array,
    B_x: jax.Array,
    B_w1: jax.Array,
    B_b1: jax.Array,
    B_w2: jax.Array,
    B_b2: jax.Array,
):
    del B_x
    B, S, D = A_x.shape
    F = B_w1.shape[1]
    assert B == 1
    f32, bf16, u32 = jnp.float32, jnp.bfloat16, jnp.uint32
    Dh = D // _H

    any_spec = pl.BlockSpec(memory_space=pl.ANY)
    s_shape = (S // 128, S // 128, 128, 128)
    scratch = [
        pltpu.VMEM((S, D), bf16),
        pltpu.VMEM((D, 3 * D + _WPAD), bf16),
        pltpu.VMEM((D, D), bf16),
        pltpu.VMEM((D, F), bf16),
        pltpu.VMEM((F,), bf16),
        pltpu.VMEM((F, D), bf16),
        pltpu.VMEM((D,), bf16),
        pltpu.VMEM((S // 2, D), u32),
        pltpu.VMEM((S // 2, 3 * D), u32),
        pltpu.VMEM((D + 64, S), u32),
        pltpu.VMEM((D, S), f32),
        pltpu.VMEM(s_shape, f32),
        pltpu.VMEM(s_shape, f32),
        pltpu.VMEM((8, S), f32),
        pltpu.VMEM((8, S), f32),
        pltpu.VMEM((S // 2, 128), u32),
        pltpu.VMEM((S // 2, 128), u32),
        pltpu.VMEM((Dh // 2, S), u32),
        pltpu.VMEM((Dh // 2, S), u32),
        pltpu.VMEM((Dh // 2, S), u32),
        pltpu.VMEM((Dh // 2, S), u32),
        pltpu.VMEM((Dh, S), f32),
        pltpu.VMEM((Dh, S), f32),
        pltpu.VMEM((8, 128), u32),
        pltpu.VMEM((2, _TM3, D), f32),
        pltpu.VMEM((_TM3 // 2, D), u32),
        pltpu.VMEM((2, _TM3, D), bf16),
        pltpu.SemaphoreType.DMA((S // _XP,)),
        pltpu.SemaphoreType.DMA((3 * D // _CW + 5 + _CW // _CW0,)),
        pltpu.SemaphoreType.DMA((2,)),
    ]
    return pl.pallas_call(
        functools.partial(_kernel, S=S, D=D, F=F),
        out_shape=jax.ShapeDtypeStruct((B, S, D), bf16),
        in_specs=[any_spec] * 7,
        out_specs=any_spec,
        scratch_shapes=scratch,
        compiler_params=pltpu.CompilerParams(
            vmem_limit_bytes=120 * 1024 * 1024,
            disable_bounds_checks=True,
            disable_semaphore_checks=True),
    )(A_x, A_wqkv, A_wo, B_w1, B_b1, B_w2, B_b2)
```

```python
import functools
import math

import jax
import jax.numpy as jnp
from jax import lax
import jax.experimental.pallas as pl
import jax.experimental.pallas.tpu as pltpu

_EPS = 1e-5
_H = 32
_TM1 = 512
_CW = 768
_CW0 = 256
_XP = 128
_TM3 = 128
_FC = 512
_QKC = 512
_KP = 512
_WPAD = 128


def _layernorm(x):
    m = jnp.mean(x, axis=-1, keepdims=True)
    xc = x - m
    v = jnp.mean(xc * xc, axis=-1, keepdims=True)
    return xc * lax.rsqrt(v + _EPS)


def _pack(x):
    return pltpu.bitcast(x, jnp.uint32)


def _unpack(x):
    return pltpu.bitcast(x, jnp.bfloat16)


def _zero_after(x):
    return jnp.minimum(jnp.abs(x), 0.0)


def _ds(start, size, align):
    if not isinstance(start, int):
        start = pl.multiple_of(start, align)
    return pl.ds(start, size)


def _kernel(x_hbm, wqkv_hbm, wo_hbm, w1_hbm, b1_hbm, w2_hbm, b2_hbm, out_hbm,
            x_v, wqkv_v, wo_v, w1_v, b1_v, w2_v, b2_v,
            y1_s, nat_s, qvt_s, ot_s, s_a, s_b, m_a, m_b,
            kc_a, kc_b, qc_a, qc_b, vc_a, vc_b, zero_s, h_s, y3_s, out_v,
            sem_x, sem_w, sem_o, *, S, D, F):
    f32, bf16 = jnp.float32, jnp.bfloat16
    Dh = D // _H
    nxp = S // _XP
    ppb = _TM1 // _XP
    ncw = 3 * D // _CW
    nsub0 = _CW // _CW0
    n1 = (S // _TM1) * ncw
    n3 = S // _TM3
    dt = D // 128
    tpw = _CW // 128
    assert ncw == ppb == 4 and _CW <= D and _TM3 == 128 and 4 * Dh == 128

    def x_copy(i):
        rows = _ds(i * _XP, _XP, _XP)
        return pltpu.make_async_copy(
            x_hbm.at[0, rows, :], x_v.at[rows, :], sem_x.at[i])

    def wqkv_copy(c):
        cols = _ds(c * _CW, _CW, 128)
        return pltpu.make_async_copy(
            wqkv_hbm.at[:, cols], wqkv_v.at[:, cols], sem_w.at[c])

    def w0_copy(j):
        cols = _ds(j * _CW0, _CW0, 128)
        return pltpu.make_async_copy(
            wqkv_hbm.at[:, cols], wqkv_v.at[:, cols], sem_w.at[ncw + 5 + j])

    late_copies = [
        pltpu.make_async_copy(wo_hbm, wo_v, sem_w.at[ncw]),
        pltpu.make_async_copy(w1_hbm, w1_v, sem_w.at[ncw + 1]),
        pltpu.make_async_copy(w2_hbm, w2_v, sem_w.at[ncw + 2]),
        pltpu.make_async_copy(b1_hbm, b1_v, sem_w.at[ncw + 3]),
        pltpu.make_async_copy(b2_hbm, b2_v, sem_w.at[ncw + 4]),
    ]

    for i in range(ppb):
        x_copy(i).start()
    w0_copy(0).start()
    zero_s[...] = jnp.zeros((8, 128), jnp.uint32)

    qscale = (Dh ** -0.5) * math.log2(math.e)

    def ln1(p):
        y = _layernorm(x_v[_ds(p * _XP, _XP, _XP), :].astype(f32))
        y1_s[_ds(p * (_XP // 2), _XP // 2, _XP // 2), :] = _pack(
            y.astype(bf16))

    def ln1_first(p, carry):
        x_copy(p).wait()
        ln1(p)
        return carry

    def transpose_tile(i, g):
        is_k = jnp.logical_and(g >= dt, g < 2 * dt)
        tt = jnp.where(is_k, 2 * dt, jnp.where(g < dt, g, g - dt))
        hrows = _ds(i * (_TM1 // 2), _TM1 // 2, _TM1 // 2)
        r = _unpack(nat_s[hrows, _ds(g * 128, 128, 128)])
        qvt_s[_ds(tt * 64, 64, 64), _ds(i * _TM1, _TM1, _TM1)] = _pack(r.T)

    def phase1_start(j, carry):
        w0_copy(j).wait()

        @pl.when(j == nsub0 - 1)
        def _():
            x_copy(ppb).wait()

        cols = _ds(j * _CW0, _CW0, 128)
        res = jnp.dot(_unpack(y1_s[0:_TM1 // 2, :]), wqkv_v[:, cols],
                      preferred_element_type=f32) * qscale
        nat_s[0:_TM1 // 2, cols] = _pack(res.astype(bf16))
        ln1(jnp.where(j == nsub0 - 1, ppb, ppb - 1))

        @pl.when(j == 0)
        def _():
            wqkv_copy(1).start()
            x_copy(ppb + 1).start()

        @pl.when(j == nsub0 - 1)
        def _():
            wqkv_copy(2).start()
            x_copy(ppb + 2).start()
        return carry

    def phase1(t, carry):
        i = t >> 2
        c = t & 3

        @pl.when(t < ncw)
        def _():
            wqkv_copy(t).wait()

        @pl.when(t + ppb < nxp)
        def _():
            x_copy(t + ppb).wait()

        for j in range(tpw):
            transpose_tile((t - 1) >> 2, ((t - 1) & 3) * tpw + j)
        hrows = _ds(i * (_TM1 // 2), _TM1 // 2, _TM1 // 2)
        res = jnp.dot(_unpack(y1_s[hrows, :]),
                      wqkv_v[:, _ds(c * _CW, _CW, 128)],
                      preferred_element_type=f32)
        for j in range(tpw):
            g = c * tpw + j
            r = res[:, j * 128:(j + 1) * 128] * jnp.where(g < dt, qscale, 1.0)
            nat_s[hrows, _ds(g * 128, 128, 128)] = _pack(r.astype(bf16))
        ln1(jnp.minimum(t + ppb, nxp - 1))

        @pl.when(t + 2 < ncw)
        def _():
            wqkv_copy(t + 2).start()

        @pl.when(t + ppb + 2 < nxp)
        def _():
            x_copy(t + ppb + 2).start()
        return carry

    lax.fori_loop(0, ppb, ln1_first, 0)
    for j in range(1, nsub0):
        w0_copy(j).start()
    x_copy(ppb).start()
    lax.fori_loop(0, nsub0, phase1_start, 0)
    lax.fori_loop(1, n1, phase1, 0)

    for c in late_copies:
        c.start()

    nkb = S // 128
    npc = S // _KP
    tpc = _QKC // 128
    ktp = _KP // 128
    hh = Dh // 2

    def stage_piece(n, nn, hq, hv, kc, qc, vc):
        rows = _ds(n * (S // 2 // nn), S // 2 // nn, S // 2 // nn)
        cols = _ds(n * (S // nn), S // nn, S // nn)
        kg = nat_s[rows, _ds(D + (hq >> 2) * 128, 128, 128)]
        kc[rows, :] = pltpu.roll(kg, (128 - (hq & 3) * Dh) & 127, 1)
        z = jnp.tile(zero_s[...], (hh // 8, S // nn // 128))
        qc[:, cols] = qvt_s[_ds(hq * hh, hh, hh), cols] | z
        vc[:, cols] = qvt_s[_ds(D // 2 + hv * hh, hh, hh), cols] | z

    def make_qk(k_tile, q_cols, s_n, m_n, hist=None):
        st = {}

        def qk(cb, kb):
            cols = _ds(cb * _QKC, _QKC, _QKC)
            if kb == 0:
                st['w'] = _unpack(jnp.concatenate(
                    [q_cols(cols), jnp.zeros((3 * hh, _QKC), jnp.uint32)],
                    axis=0))
            s = jnp.dot(_unpack(k_tile(kb)), st['w'],
                        preferred_element_type=f32)
            if hist is not None:
                hist.append(s[:, 0:128])
            for t in range(tpc):
                s_n[cb * tpc + t, kb] = s[:, t * 128:(t + 1) * 128]
            mm = jnp.max(s.reshape(16, 8, _QKC), axis=0)
            st['m'] = mm if kb == 0 else jnp.maximum(st['m'], mm)
            if kb == nkb - 1:
                m_n[:, cols] = jnp.broadcast_to(
                    jnp.max(st['m'], axis=0, keepdims=True), (8, _QKC))
        return qk

    def make_sm(h, v_cols, s_c, m_c, hist=None, pace=False):
        st = {}

        def sm(ct, pc):
            cols = _ds(ct * 128, 128, 128)
            mv = m_c[:, cols]
            if pace:
                src = hist[-2]
                mvs = jnp.stack([
                    mv + _zero_after(src[(7 - r) * 16:(7 - r) * 16 + 8])
                    for r in range(8)], axis=0)
                mv = mvs[None, :, None]
            p = jnp.exp2(
                s_c[ct, pc * ktp:(pc + 1) * ktp].reshape(ktp, 8, 2, 8, 128)
                - mv)
            pairs = p[:, :, 0] + p[:, :, 1]
            for r in reversed(range(8)):
                first = pc == 0 and r == 7
                st['l'] = pairs[:, r] if first else st['l'] + pairs[:, r]
            o = jnp.dot(_unpack(v_cols(slice(pc * _KP, (pc + 1) * _KP))),
                        p.reshape(_KP, 128).astype(bf16),
                        preferred_element_type=f32)
            st['o'] = o if pc == 0 else o + st['o']
            if pc == npc - 1:
                l = st['l'][0]
                for t in range(1, ktp):
                    l = l + st['l'][t]
                ot_s[_ds(h * Dh, Dh, Dh), cols] = (
                    st['o'] / jnp.sum(l, axis=0, keepdims=True))
        return sm

    def step(h, cur, nxt, hist, pace):
        (s_c, m_c, kc, qc, vc), (s_n, m_n, kn, qn, vn) = cur, nxt
        qk = make_qk(lambda kb: kc[kb * 64:(kb + 1) * 64, :],
                     lambda cols: qc[:, cols], s_n, m_n, hist)
        sm = make_sm(h, lambda cols: vc[:, cols], s_c, m_c, hist, pace)
        qk_ids = [(cb, kb) for cb in range(S // _QKC) for kb in range(nkb)]
        sm_ids = [(ct, pc) for ct in range(S // 128) for pc in range(npc)]
        assert len(qk_ids) == len(sm_ids)
        hq = jnp.minimum(h + 2, _H - 1)
        for n, (a, b) in enumerate(zip(qk_ids, sm_ids)):
            qk(*a)
            sm(*b)
            if n % 3 == 2 and n // 3 < 16:
                stage_piece(n // 3, 16, hq, h + 1, kn, qn, vn)

    buf_a = (s_a, m_a, kc_a, qc_a, vc_a)
    buf_b = (s_b, m_b, kc_b, qc_b, vc_b)

    def first_heads(cb, carry):
        def k_tile(kb):
            return nat_s[kb * 64:(kb + 1) * 64, D:D + 128]

        hist = []
        qk0 = make_qk(k_tile, lambda cols: qvt_s[0:hh, cols], s_a, m_a, hist)
        qk1 = make_qk(lambda kb: pltpu.roll(k_tile(kb), 128 - Dh, 1),
                      lambda cols: qvt_s[hh:2 * hh, cols], s_b, m_b, hist)
        sm0 = make_sm(0, lambda cols: qvt_s[D // 2:D // 2 + hh, cols],
                      s_a, m_a, hist, True)
        g0 = (ncw - 1) * tpw
        for kb in range(nkb):
            qk0(cb, kb)
            if kb == 1:
                stage_piece(cb, S // _QKC, 2, 1, kc_b, qc_b, vc_b)
            if kb == 5:
                transpose_tile(S // _TM1 - 1, g0 + cb)
            if kb == 9:
                transpose_tile(S // _TM1 - 1,
                               g0 + jnp.minimum(cb + 4, tpw - 1))
        qk1(cb, 0)
        for kb in range(1, nkb):
            qk1(cb, kb)
            sm0(cb * tpc + (kb - 1) // npc, (kb - 1) % npc)
        sm0(cb * tpc + tpc - 1, npc - 1)
        return carry

    def phase2(i, carry):
        hist = []
        step(2 * i + 1, buf_b, buf_a, hist, False)
        step(2 * i + 2, buf_a, buf_b, hist, True)
        return carry

    lax.fori_loop(0, S // _QKC, first_heads, 0)
    lax.fori_loop(0, (_H - 2) // 2, phase2, 0)

    for c in late_copies:
        c.wait()

    def out_copy(i):
        return pltpu.make_async_copy(
            out_v.at[i & 1], out_hbm.at[0, _ds(i * _TM3, _TM3, _TM3), :],
            sem_o.at[i & 1])

    def finish_a(h, slot):
        h_s[slot] = h
        y3_s[...] = _pack(_layernorm(_layernorm(h)).astype(bf16))

    def stage_a(i, slot):
        rows = _ds(i * _TM3, _TM3, _TM3)
        o = ot_s[:, rows].T.astype(bf16)
        finish_a(x_v[rows, :].astype(f32) + jnp.dot(
            o, wo_v[...], preferred_element_type=f32), slot)

    sm_last = make_sm(_H - 1, lambda cols: vc_b[:, cols], s_b, m_b)
    k0 = D - 128
    o0 = ot_s[0:k0, 0:_TM3].T.astype(bf16)
    hs = []
    for n in range(dt):
        cs = slice(n * 128, (n + 1) * 128)
        hs.append(x_v[0:_TM3, cs].astype(f32) + jnp.dot(
            o0, wo_v[0:k0, cs], preferred_element_type=f32))
        sm_last(n // npc, n % npc)
    o1 = ot_s[k0:D, 0:_TM3].T.astype(bf16)
    finish_a(jnp.concatenate(hs, axis=1) + jnp.dot(
        o1, wo_v[k0:D, :], preferred_element_type=f32), 0)

    def mlp_block(i, last):
        sm31 = make_sm(_H - 1, lambda cols: vc_b[:, cols], s_b, m_b)
        y = _unpack(y3_s[...])
        gs = []
        for c in range(F // _FC):
            a = jnp.dot(y, w1_v[:, c * _FC:(c + 1) * _FC],
                        preferred_element_type=f32)
            a = a + b1_v[pl.ds(c * _FC, _FC)].astype(f32).reshape(1, _FC)
            gs.append(jax.nn.gelu(a, approximate=True).astype(bf16))
            if not last and 1 <= c <= npc:
                sm31(jnp.minimum(i + 2, n3 - 1), c - 1)
        if not last:
            stage_a(i + 1, (i + 1) & 1)
        g = jnp.concatenate(gs, axis=1)
        r = jnp.dot(g, w2_v[...], preferred_element_type=f32)
        res = h_s[i & 1] + (r + b2_v[...].astype(f32).reshape(1, D))
        out_v[i & 1] = res.astype(bf16)
        out_copy(i).start()

    def phase3(i, carry):
        @pl.when(i >= 2)
        def _():
            out_copy(i - 2).wait()

        mlp_block(i, False)
        return carry

    lax.fori_loop(0, n3 - 1, phase3, 0)
    out_copy(n3 - 3).wait()
    mlp_block(n3 - 1, True)
    out_copy(n3 - 2).wait()
    out_copy(n3 - 1).wait()


@jax.jit
def pallas_sequential_preLN__softmax_full_mha__mixer_channel_mlp__prompt_kernel(
    A_x: jax.Array,
    A_wqkv: jax.Array,
    A_wo: jax.Array,
    B_x: jax.Array,
    B_w1: jax.Array,
    B_b1: jax.Array,
    B_w2: jax.Array,
    B_b2: jax.Array,
):
    del B_x
    B, S, D = A_x.shape
    F = B_w1.shape[1]
    assert B == 1
    f32, bf16, u32 = jnp.float32, jnp.bfloat16, jnp.uint32
    Dh = D // _H

    any_spec = pl.BlockSpec(memory_space=pl.ANY)
    s_shape = (S // 128, S // 128, 128, 128)
    scratch = [
        pltpu.VMEM((S, D), bf16),
        pltpu.VMEM((D, 3 * D + _WPAD), bf16),
        pltpu.VMEM((D, D), bf16),
        pltpu.VMEM((D, F), bf16),
        pltpu.VMEM((F,), bf16),
        pltpu.VMEM((F, D), bf16),
        pltpu.VMEM((D,), bf16),
        pltpu.VMEM((S // 2, D), u32),
        pltpu.VMEM((S // 2, 3 * D), u32),
        pltpu.VMEM((D + 64, S), u32),
        pltpu.VMEM((D, S), f32),
        pltpu.VMEM(s_shape, f32),
        pltpu.VMEM(s_shape, f32),
        pltpu.VMEM((8, S), f32),
        pltpu.VMEM((8, S), f32),
        pltpu.VMEM((S // 2, 128), u32),
        pltpu.VMEM((S // 2, 128), u32),
        pltpu.VMEM((Dh // 2, S), u32),
        pltpu.VMEM((Dh // 2, S), u32),
        pltpu.VMEM((Dh // 2, S), u32),
        pltpu.VMEM((Dh // 2, S), u32),
        pltpu.VMEM((8, 128), u32),
        pltpu.VMEM((2, _TM3, D), f32),
        pltpu.VMEM((_TM3 // 2, D), u32),
        pltpu.VMEM((2, _TM3, D), bf16),
        pltpu.SemaphoreType.DMA((S // _XP,)),
        pltpu.SemaphoreType.DMA((3 * D // _CW + 5 + _CW // _CW0,)),
        pltpu.SemaphoreType.DMA((2,)),
    ]
    return pl.pallas_call(
        functools.partial(_kernel, S=S, D=D, F=F),
        out_shape=jax.ShapeDtypeStruct((B, S, D), bf16),
        in_specs=[any_spec] * 7,
        out_specs=any_spec,
        scratch_shapes=scratch,
        compiler_params=pltpu.CompilerParams(
            vmem_limit_bytes=120 * 1024 * 1024,
            disable_bounds_checks=True,
            disable_semaphore_checks=True),
    )(A_x, A_wqkv, A_wo, B_w1, B_b1, B_w2, B_b2)
```
